```python
import os as _os
_os.environ.setdefault("JAX_PLATFORMS", "cpu")
import jax
import jax.numpy as jnp

def _softmax(x, axis=-1):
    return jax.nn.softmax(x, axis=axis)
def _gelu(x):
    return jax.nn.gelu(x, approximate=True)
def _silu(x):
    return jax.nn.silu(x)
def _sigmoid(x):
    return jax.nn.sigmoid(x)
def _layernorm(x, axis=-1, eps=1e-5):
    m = jnp.mean(x, axis=axis, keepdims=True)
    v = jnp.var(x, axis=axis, keepdims=True)
    return (x - m) / jnp.sqrt(v + eps)
def _scatter_add(tgt, idx, src, axis=0):
    return tgt.at[idx].add(src)
def _segment_sum(src, seg, n):
    return jax.ops.segment_sum(src, seg, n)
class _Rng:
    def __init__(self, key):
        self._k = key
    def _next(self):
        self._k, sub = jax.random.split(self._k)
        return sub
    def normal(self, shape):
        return jax.random.normal(self._next(), shape, dtype=jnp.bfloat16)
    def randint(self, lo, hi, shape):
        return jax.random.randint(self._next(), shape, lo, hi, dtype=jnp.int32)
    def uniform(self, shape, lo=0.0, hi=1.0):
        return jax.random.uniform(self._next(), shape, jnp.bfloat16, lo, hi)
    def permutation(self, n):
        return jax.random.permutation(self._next(), n)


kernel_name = 'sequential_preLN__softmax_full_mha__dense_activation_gelu__prompt'

def setup_inputs():
    _rng = _Rng(jax.random.key(int.from_bytes(__import__("os").urandom(4), "little")))
    _w = (lambda a: (lambda t: t.astype(jnp.bfloat16) if jnp.issubdtype(t.dtype, jnp.floating) else t)(jnp.asarray(a)))
    def _A_setup():
        B, S, D = 1, 2048, 640
        return {
            "x": _w((lambda *s: _rng.normal(s) * 0.05)(B, S, D)),
            "wqkv": _w((lambda *s: _rng.normal(s) * 0.05)(D, 3 * D)),
            "wo": _w((lambda *s: _rng.normal(s) * 0.05)(D, D)),
        }
    _A_in = _A_setup()

    def _B_setup():
        B, S, D, F = 1, 2048, 640, 1536
        return {
            "x": _w((lambda *s: _rng.normal(s) * 0.05)(B, S, D)),
            "w1": _w((lambda *s: _rng.normal(s) * 0.4)(D, F) * (D ** -0.5)),
            "b1": _w((lambda *s: _rng.normal(s) * 0.4)(F) * 0.01),
            "w2": _w((lambda *s: _rng.normal(s) * 0.4)(F, D) * (F ** -0.5)),
            "b2": _w((lambda *s: _rng.normal(s) * 0.05)(D) * 0.01),
        }
    _B_in = _B_setup()

    return {
        "A_x": _A_in["x"],
        "A_wqkv": _A_in["wqkv"],
        "A_wo": _A_in["wo"],
        "B_x": _B_in["x"],
        "B_w1": _B_in["w1"],
        "B_b1": _B_in["b1"],
        "B_w2": _B_in["w2"],
        "B_b2": _B_in["b2"],
    }

def reference(A_x, A_wqkv, A_wo, B_x, B_w1, B_b1, B_w2, B_b2):
    def _A_ref(x, wqkv, wo):
        B, S, D = x.shape
        H = 32; Dh = D // H
        qkv = (lambda x, *d: x.transpose(*d))((x @ wqkv).reshape(B, S, 3, H, Dh), 2, 0, 3, 1, 4)
        q, k, v = qkv[0], qkv[1], qkv[2]
        scale = Dh ** -0.5
        scores = jnp.einsum("bhqd,bhkd->bhqk", q, k) * scale
        p = _softmax(scores, axis=-1)
        o = jnp.einsum("bhqk,bhkd->bhqd", p, v)
        return (lambda x, *d: x.transpose(*d))(o, 0, 2, 1, 3).reshape(B, S, D) @ wo

    def _B_ref(x, w1, b1, w2, b2):
        h = jnp.einsum("bsd,df->bsf", x, w1) + b1
        h = _gelu(h)
        return jnp.einsum("bsf,fd->bsd", h, w2) + b2

    x = A_x
    h = x + _A_ref(_layernorm(x, axis=-1), A_wqkv, A_wo)
    h2 = h + _B_ref(_layernorm(h, axis=-1), B_w1, B_b1, B_w2, B_b2)
    return h2
```

```python
import functools
import math
import jax
import jax.numpy as jnp
from jax import lax
import jax.experimental.pallas as pl
import jax.experimental.pallas.tpu as pltpu

S = 2048
D = 640
H = 32
DH = 20
F = 1536
NT5 = D // 128
NTILE = 9
VR = 24
DV = H * VR
TQ = 512
NQ = S // TQ
NU = NQ * H
EPS = 1e-5
QSCALE = (DH ** -0.5) * math.log2(math.e)

NT = (((1,), (1,)), ((), ()))
TN = (((0,), (0,)), ((), ()))
f32 = jnp.float32
bf16 = jnp.bfloat16


def _ln(x):
    m = jnp.mean(x, axis=-1, keepdims=True)
    xc = x - m
    v = jnp.mean(xc * xc, axis=-1, keepdims=True)
    return xc * lax.rsqrt(v + EPS)


def _gelu(x):
    c = math.sqrt(2.0 / math.pi)
    return 0.5 * x * (1.0 + jnp.tanh(c * (x + 0.044715 * (x * x * x))))


def kernel(x_hbm, wqkv_hbm, wo_hbm, w1_hbm, w2_hbm, b1_ref, b2_ref, o_hbm,
           x_s, wqkv_s, wo_s, w1_s, w2_s, k_s, q_s, vT_s, sA, sB, oT_s, out_s,
           sem_x, sem_w, sem_o, *, kc, sig, t1, t3, scopes):
    scope = jax.named_scope if scopes else (lambda name: _Null())
    n1 = S // t1
    nsteps = S // kc

    def x_copy(t):
        rows = pl.ds(t * t1, t1) if isinstance(t, int) else pl.ds(pl.multiple_of(t * t1, t1), t1)
        return pltpu.make_async_copy(x_hbm.at[rows, :], x_s.at[rows, :], sem_x.at[t])

    wqkv_copy = pltpu.make_async_copy(wqkv_hbm, wqkv_s, sem_w.at[0])
    wo_copy = pltpu.make_async_copy(wo_hbm, wo_s, sem_w.at[1])
    w1_copy = pltpu.make_async_copy(w1_hbm, w1_s, sem_w.at[2])
    w2_copy = pltpu.make_async_copy(w2_hbm, w2_s, sem_w.at[3])

    x_copy(0).start()
    wqkv_copy.start()
    for t in range(1, n1):
        x_copy(t).start()
    wo_copy.start()
    w1_copy.start()
    w2_copy.start()
    wqkv_copy.wait()

    def p1(t, carry):
        x_copy(t).wait()
        rows = pl.ds(pl.multiple_of(t * t1, t1), t1)
        xn = _ln(x_s[rows, :].astype(f32)).astype(bf16)
        hi = lax.broadcasted_iota(jnp.int32, (t1, 128), 1) >= 64
        for dst, base, scl in ((q_s, 0, QSCALE), (k_s, D, None)):
            y = jnp.dot(xn, wqkv_s[:, base:base + D], preferred_element_type=f32)
            if scl is not None:
                y = y * scl
            tiles = [y[:, 128 * j:128 * (j + 1)] for j in range(NT5)]
            for j in range(NT5):
                dst[j, rows, :] = tiles[j].astype(bf16)
            for j in range(NT5 - 1):
                dst[NT5 + j, rows, :] = jnp.where(hi, tiles[j], tiles[j + 1]).astype(bf16)
        v = jnp.dot(xn, wqkv_s[:, 2 * D:3 * D], preferred_element_type=f32)
        vT = v.astype(bf16).T.astype(f32)
        lo4 = lax.broadcasted_iota(jnp.int32, (8, t1), 0) < 4
        for p in range(H // 2):
            vT_s[48 * p:48 * p + 16, rows] = vT[40 * p:40 * p + 16]
            mid = vT[40 * p + 16:40 * p + 24]
            vT_s[48 * p + 16:48 * p + 24, rows] = jnp.where(lo4, mid, 1.0)
            vT_s[48 * p + 24:48 * p + 32, rows] = jnp.where(lo4, 1.0, mid)
            vT_s[48 * p + 32:48 * p + 48, rows] = vT[40 * p + 24:40 * p + 40]
        return carry

    with scope("phase1"):
        lax.fori_loop(0, n1, p1, 0)

    def unit_q(u):
        if isinstance(u, int):
            u = min(u, NU - 1)
            qb, h = divmod(u, H)
            off = (h * DH) % 128
            tile = (h * DH) // 128 + (NT5 if off > 128 - DH else 0)
            qrows = pl.ds(qb * TQ, TQ)
        else:
            u = jnp.minimum(u, NU - 1)
            qb = u // H
            h = u - qb * H
            off = (h * DH) % 128
            tile = (h * DH) // 128 + jnp.where(off > 128 - DH, NT5, 0)
            qrows = pl.ds(pl.multiple_of(qb * TQ, TQ), TQ)
        lane = lax.broadcasted_iota(jnp.int32, (TQ, 128), 1)
        msk = ((lane - off + 128) & 127) < DH
        qm = jnp.where(msk, q_s[tile, qrows, :], jnp.zeros((), bf16))
        return qm, tile

    def stepA(qm, tile, c, sbuf, m8):
        krows = pl.ds(c * kc, kc)
        s = lax.dot_general(k_s[tile, krows, :], qm, NT, preferred_element_type=f32)
        sbuf[krows, :] = s
        mm = jnp.max(s.reshape(kc // 8, 8, TQ), axis=0)
        return mm if m8 is None else jnp.maximum(m8, mm)

    def stepB(vrow0, c, sbuf, m, acc):
        krows = pl.ds(c * kc, kc)
        p = jnp.exp2(sbuf[krows, :] - m).astype(bf16)
        r = jnp.dot(vT_s[pl.ds(vrow0, VR), krows], p, preferred_element_type=f32)
        return r if acc is None else acc + r

    def finish(m8):
        return jnp.max(m8, axis=0, keepdims=True)

    with scope("prologue"):
        qm, tile = unit_q(0)
        m8 = None
        for c in range(nsteps):
            m8 = stepA(qm, tile, c, sA, m8)
        m_cur0 = finish(m8)
        qm, tile = unit_q(1)
        m8 = None
        for c in range(sig):
            m8 = stepA(qm, tile, c, sB, m8)
        m8_next0 = m8 if sig > 0 else jnp.full((8, TQ), -jnp.inf, f32)

    def body(i, carry):
        m_e, m8_o = carry
        pr = i % (H // 2)
        vrow_e = pl.multiple_of(pr * 48, 8)
        vrow_o = pl.multiple_of(pr * 48 + 24, 8)
        orow = pl.multiple_of(pr * 40, 8)
        qm1, tile1 = unit_q(2 * i + 1)
        qm2, tile2 = unit_q(2 * i + 2)
        qm3, tile3 = unit_q(2 * i + 3)
        acc_e = None
        acc_o = None
        m8_2 = None
        m8_3 = None
        m_o = None
        mid_e = None
        lo4 = lax.broadcasted_iota(jnp.int32, (8, TQ), 0) < 4
        for n in range(2 * nsteps):
            a = n + sig
            if a < nsteps:
                m8_o = stepA(qm1, tile1, a, sB, m8_o)
                if a == nsteps - 1:
                    m_o = finish(m8_o)
            elif a < 2 * nsteps:
                m8_2 = stepA(qm2, tile2, a - nsteps, sA, m8_2)
            else:
                m8_3 = stepA(qm3, tile3, a - 2 * nsteps, sB, m8_3)
            if n < nsteps:
                acc_e = stepB(vrow_e, n, sA, m_e, acc_e)
                if n == nsteps - 1:
                    o = acc_e * (1.0 / acc_e[DH:DH + 1, :])
                    oT_s[pl.ds(orow, 16), :] = o[0:16]
                    mid_e = o[16:24]
            else:
                acc_o = stepB(vrow_o, n - nsteps, sB, m_o, acc_o)
                if n == 2 * nsteps - 1:
                    o = acc_o * (1.0 / acc_o[0:1, :])
                    oT_s[pl.ds(orow + 16, 8), :] = jnp.where(lo4, mid_e, o[0:8])
                    oT_s[pl.ds(orow + 24, 16), :] = o[8:24]
        if sig == 0:
            m8_3 = jnp.full((8, TQ), -jnp.inf, f32)
        return finish(m8_2), m8_3

    n3 = TQ // t3

    def out_copy(slot, row0):
        return pltpu.make_async_copy(out_s.at[slot], o_hbm.at[pl.ds(row0, t3), :], sem_o.at[slot])

    def qblock(qb, carry):
        with scope("attnloop"):
            carry = lax.fori_loop(qb * (H // 2), (qb + 1) * (H // 2), body, carry)

        @pl.when(qb == 0)
        def _():
            wo_copy.wait()
            w1_copy.wait()
            w2_copy.wait()

        def p3(t, c):
            g = qb * n3 + t
            slot = g % 2
            row0 = pl.multiple_of(g * t3, t3)

            @pl.when(g >= 2)
            def _():
                out_copy(slot, pl.multiple_of((g - 2) * t3, t3)).wait()

            cols = pl.ds(pl.multiple_of(t * t3, t3), t3)
            oT = oT_s[:, cols].astype(bf16)
            attn = lax.dot_general(oT, wo_s[...], TN, preferred_element_type=f32)
            hres = x_s[pl.ds(row0, t3), :].astype(f32) + attn
            hn = _ln(hres).astype(bf16)
            a = jnp.dot(hn, w1_s[...], preferred_element_type=f32) + b1_ref[...].astype(f32)
            a = _gelu(a).astype(bf16)
            y = jnp.dot(a, w2_s[...], preferred_element_type=f32) + b2_ref[...].astype(f32)
            out_s[slot] = (hres + y).astype(bf16)
            out_copy(slot, row0).start()
            return c

        with scope("phase3"):
            lax.fori_loop(0, n3, p3, 0)
        return carry

    lax.fori_loop(0, NQ, qblock, (m_cur0, m8_next0))
    ng = NQ * n3
    out_copy((ng - 2) % 2, (ng - 2) * t3).wait()
    out_copy((ng - 1) % 2, (ng - 1) * t3).wait()


class _Null:
    def __enter__(self):
        return self
    def __exit__(self, *a):
        return False


def make(kc=128, sig=1, t1=512, t3=256, scopes=False):
    @jax.jit
    def fn(A_x, A_wqkv, A_wo, B_x, B_w1, B_b1, B_w2, B_b2):
        x = A_x.reshape(S, D)
        b1 = B_b1.reshape(1, F)
        b2 = B_b2.reshape(1, D)
        anyspec = pl.BlockSpec(memory_space=pl.ANY)
        vm = pl.BlockSpec(memory_space=pltpu.VMEM)
        out = pl.pallas_call(
            functools.partial(kernel, kc=kc, sig=sig, t1=t1, t3=t3, scopes=scopes),
            in_specs=[anyspec] * 5 + [vm, vm],
            out_specs=anyspec,
            out_shape=jax.ShapeDtypeStruct((S, D), bf16),
            scratch_shapes=[
                pltpu.VMEM((S, D), bf16),
                pltpu.VMEM((D, 3 * D), bf16),
                pltpu.VMEM((D, D), bf16),
                pltpu.VMEM((D, F), bf16),
                pltpu.VMEM((F, D), bf16),
                pltpu.VMEM((NTILE, S, 128), bf16),
                pltpu.VMEM((NTILE, S, 128), bf16),
                pltpu.VMEM((DV, S), f32),
                pltpu.VMEM((S, TQ), f32),
                pltpu.VMEM((S, TQ), f32),
                pltpu.VMEM((D, TQ), f32),
                pltpu.VMEM((2, t3, D), bf16),
                pltpu.SemaphoreType.DMA((S // t1,)),
                pltpu.SemaphoreType.DMA((4,)),
                pltpu.SemaphoreType.DMA((2,)),
            ],
            compiler_params=pltpu.CompilerParams(vmem_limit_bytes=100 * 1024 * 1024),
        )(x, A_wqkv, A_wo, B_w1, B_w2, b1, b2)
        return out.reshape(1, S, D)
    return fn


_fn = make()


@jax.jit
def pallas_sequential_preLN__softmax_full_mha__dense_activation_gelu__prompt_kernel(
    A_x: jax.Array,
    A_wqkv: jax.Array,
    A_wo: jax.Array,
    B_x: jax.Array,
    B_w1: jax.Array,
    B_b1: jax.Array,
    B_w2: jax.Array,
    B_b2: jax.Array,
):
    return _fn(A_x, A_wqkv, A_wo, B_x, B_w1, B_b1, B_w2, B_b2)
```

```python
import functools
import math
import jax
import jax.numpy as jnp
from jax import lax
import jax.experimental.pallas as pl
import jax.experimental.pallas.tpu as pltpu

S = 2048
D = 640
H = 32
DH = 20
F = 1536
NT5 = D // 128
NTILE = 9
VR = 24
DV = H * VR
TQ = 512
NQ = S // TQ
KC = 128
NSTEP = S // KC
EPS = 1e-5
QSCALE = (DH ** -0.5) * math.log2(math.e)

TN = (((0,), (0,)), ((), ()))
f32 = jnp.float32
bf16 = jnp.bfloat16


def _ln(x):
    m = jnp.mean(x, axis=-1, keepdims=True)
    xc = x - m
    v = jnp.mean(xc * xc, axis=-1, keepdims=True)
    return xc * lax.rsqrt(v + EPS)


def _gelu(x):
    c = math.sqrt(2.0 / math.pi)
    return 0.5 * x * (1.0 + jnp.tanh(c * (x + 0.044715 * (x * x * x))))


class _Null:
    def __enter__(self):
        return self

    def __exit__(self, *a):
        return False


def kernel(x_hbm, wqkv_hbm, wo_hbm, w1_hbm, w2_hbm, b1_hbm, b2_hbm, o_hbm,
           x_s, wqkv_s, wo_s, w1_s, w2_s, k_s, qT_s, vT_s, sA, sB, oT_s, out_s, b1_ref, b2_ref,
           sem_x, sem_w, sem_o, *, sig, t1, t3, nh3, scopes):
    scope = jax.named_scope if scopes else (lambda name: _Null())
    n1 = S // t1

    def rows_of(t, size):
        return pl.ds(t * size, size) if isinstance(t, int) else pl.ds(pl.multiple_of(t * size, size), size)

    def x_copy(t):
        rows = rows_of(t, t1)
        return pltpu.make_async_copy(x_hbm.at[rows, :], x_s.at[rows, :], sem_x.at[t])

    def wqkv_copy(j):
        cols = pl.ds(j * D, D)
        return pltpu.make_async_copy(wqkv_hbm.at[:, cols], wqkv_s.at[:, cols], sem_w.at[j])

    wo_copy = pltpu.make_async_copy(wo_hbm, wo_s, sem_w.at[3])
    w1_copy = pltpu.make_async_copy(w1_hbm, w1_s, sem_w.at[4])
    w2_copy = pltpu.make_async_copy(w2_hbm, w2_s, sem_w.at[5])

    b1_copy = pltpu.make_async_copy(b1_hbm, b1_ref, sem_w.at[6])
    b2_copy = pltpu.make_async_copy(b2_hbm, b2_ref, sem_w.at[7])

    x_copy(0).start()
    wqkv_copy(2).start()
    sB[...] = jnp.zeros((S, TQ), f32)
    oT_s[16:24, 3 * TQ:4 * TQ] = jnp.zeros((8, TQ), f32)

    def ln_chunk(t):
        return _ln(x_s[rows_of(t, t1), :].astype(f32)).astype(bf16)

    def p1_mm(xn, t, first):
        rows = rows_of(t, t1)
        if first:
            wqkv_copy(2).wait()
            wqkv_copy(0).start()
        v = jnp.dot(xn, wqkv_s[:, 2 * D:3 * D], preferred_element_type=f32).astype(bf16)
        if first:
            wqkv_copy(0).wait()
            wqkv_copy(1).start()
            x_copy(1).start()
        q = (jnp.dot(xn, wqkv_s[:, 0:D], preferred_element_type=f32) * QSCALE).astype(bf16)
        vT = v.T.astype(f32)
        lo4 = lax.broadcasted_iota(jnp.int32, (8, t1), 0) < 4
        for p in range(H // 2):
            vT_s[48 * p:48 * p + 16, rows] = vT[40 * p:40 * p + 16]
            mid = vT[40 * p + 16:40 * p + 24]
            vT_s[48 * p + 16:48 * p + 24, rows] = jnp.where(lo4, mid, 1.0)
            vT_s[48 * p + 24:48 * p + 32, rows] = jnp.where(lo4, 1.0, mid)
            vT_s[48 * p + 32:48 * p + 48, rows] = vT[40 * p + 24:40 * p + 40]
        if first:
            wqkv_copy(1).wait()
            x_copy(1).wait()
            for tt in range(2, n1):
                x_copy(tt).start()
        y = jnp.dot(xn, wqkv_s[:, D:2 * D], preferred_element_type=f32)
        qT_s[:, rows] = q.T
        hi = lax.broadcasted_iota(jnp.int32, (t1, 128), 1) >= 64
        tiles = [y[:, 128 * j:128 * (j + 1)] for j in range(NT5)]
        for j in range(NT5):
            k_s[j, rows, :] = tiles[j].astype(bf16)
        for j in range(NT5 - 1):
            k_s[NT5 + j, rows, :] = jnp.where(hi, tiles[j], tiles[j + 1]).astype(bf16)

    def p1(t, xn):
        @pl.when(t + 1 < n1)
        def _():
            x_copy(t + 1).wait()
        xn_next = ln_chunk(jnp.minimum(t + 1, n1 - 1))
        p1_mm(xn, t, False)
        return xn_next

    with scope("phase1"):
        x_copy(0).wait()
        xn0 = ln_chunk(0)
        p1_mm(xn0, 0, True)
        xn1 = ln_chunk(1)
        wo_copy.start()
        w1_copy.start()
        w2_copy.start()
        b1_copy.start()
        b2_copy.start()
        lax.fori_loop(1, n1, p1, xn1)

    def unit_q(pr, par, qb):
        h = 2 * pr + par
        off = (h * DH) % 128
        t = (h * DH) // 128
        strad = off > 128 - DH
        qcols = pl.ds(qb * TQ, TQ)
        if isinstance(h, int):
            tile = t + (NT5 if strad else 0)
            ra = pl.ds(128 * t + (128 if strad else 0), 64)
            rb = pl.ds(128 * t + 64, 64)
        else:
            tile = t + jnp.where(strad, NT5, 0)
            ra = pl.ds(pl.multiple_of(128 * t + jnp.where(strad, 128, 0), 64), 64)
            rb = pl.ds(pl.multiple_of(128 * t + 64, 64), 64)
        w = jnp.concatenate([qT_s[ra, qcols], qT_s[rb, qcols]], axis=0)
        r = lax.broadcasted_iota(jnp.int32, (128, TQ), 0)
        msk = ((r - off + 128) & 127) < DH
        return jnp.where(msk, w, jnp.zeros((), bf16)), tile

    def stepA(uq, c, sbuf, m8):
        qm, tile = uq
        krows = pl.ds(c * KC, KC)
        s = jnp.dot(k_s[tile, krows, :], qm, preferred_element_type=f32)
        sbuf[krows, :] = s
        mm = jnp.max(s.reshape(KC // 8, 8, TQ), axis=0)
        return mm if m8 is None else jnp.maximum(m8, mm)

    def stepB(pr, par, c, sbuf, m, acc):
        krows = pl.ds(c * KC, KC)
        vrow = pr * 48 + 24 * par
        if not isinstance(vrow, int):
            vrow = pl.multiple_of(vrow, 8)
        p = jnp.exp2(sbuf[krows, :] - m).astype(bf16)
        r = jnp.dot(vT_s[pl.ds(vrow, VR), krows], p, preferred_element_type=f32)
        return r if acc is None else acc + r

    def finish(m8):
        return jnp.max(m8, axis=0, keepdims=True)

    def store_o(acc, pr, par, qb):
        orow = pr * 40
        if not isinstance(orow, int):
            orow = pl.multiple_of(orow, 8)
        qcols = pl.ds(qb * TQ, TQ)
        if par == 0:
            oT_s[pl.ds(orow, VR), qcols] = acc * (1.0 / acc[DH:DH + 1, :])
        else:
            o = acc * (1.0 / acc[0:1, :])
            lo4 = lax.broadcasted_iota(jnp.int32, (8, TQ), 0) < 4
            mid_e = oT_s[pl.ds(orow + 16, 8), qcols]
            oT_s[pl.ds(orow + 16, 8), qcols] = jnp.where(lo4, mid_e, o[0:8])
            oT_s[pl.ds(orow + 24, 16), qcols] = o[8:24]

    sbufs = (sA, sB)

    with scope("prologue"):
        uq = unit_q(0, 0, 0)
        m8 = None
        for c in range(sig):
            m8 = stepA(uq, c, sA, m8)
        m8_0 = m8

    def body(p, carry):
        m_prev, m8 = carry
        pn = jnp.minimum(p + 1, H // 2 - 1)
        pp = jnp.maximum(p - 1, 0)
        uq = None
        acc = None
        ms = {-1: m_prev}
        for n in range(8 * NSTEP):
            a = n + sig
            ka, ca = divmod(a, NSTEP)
            if ca == 0 or n == 0:
                uq = unit_q(p if ka < 8 else pn, (ka % 8) // 4, ka % 4)
                if ca == 0:
                    m8 = None
            m8 = stepA(uq, ca, sbufs[ka % 2], m8)
            if ca == NSTEP - 1:
                ms[ka] = finish(m8)
            kb, cb = divmod(n, NSTEP)
            kb -= 1
            pr = pp if kb < 0 else p
            par, qb = (kb % 8) // 4, kb % 4
            acc = stepB(pr, par, cb, sbufs[kb % 2], ms[kb], None if cb == 0 else acc)
            if cb == NSTEP - 1:
                store_o(acc, pr, par, qb)
        return ms[7], m8

    with scope("attnloop"):
        m_last, _ = lax.fori_loop(0, H // 2, body, (jnp.zeros((1, TQ), f32), m8_0))

    with scope("epilogue"):
        acc = None
        for c in range(NSTEP):
            acc = stepB(H // 2 - 1, 1, c, sB, m_last, acc)
        store_o(acc, H // 2 - 1, 1, NQ - 1)

    wo_copy.wait()
    w1_copy.wait()
    w2_copy.wait()
    b1_copy.wait()
    b2_copy.wait()

    ntrip = S // (t3 * nh3)

    def out_copy(g):
        slot = g % (2 * nh3)
        return pltpu.make_async_copy(out_s.at[slot], o_hbm.at[rows_of(g, t3), :], sem_o.at[slot])

    def p3(trip, c):
        @pl.when(trip >= 2)
        def _():
            for k in range(nh3):
                out_copy((trip - 2) * nh3 + k).wait()

        b1 = b1_ref[...].reshape(1, F).astype(f32)
        b2 = b2_ref[...].reshape(1, D).astype(f32)
        hres = []
        for k in range(nh3):
            rows = rows_of(trip * nh3 + k, t3)
            oT = oT_s[:, rows].astype(bf16)
            attn = lax.dot_general(oT, wo_s[...], TN, preferred_element_type=f32)
            hres.append(x_s[rows, :].astype(f32) + attn)
        act = []
        for k in range(nh3):
            hn = _ln(hres[k]).astype(bf16)
            a = jnp.dot(hn, w1_s[...], preferred_element_type=f32) + b1
            act.append(_gelu(a).astype(bf16))
        for k in range(nh3):
            g = trip * nh3 + k
            y = jnp.dot(act[k], w2_s[...], preferred_element_type=f32) + b2
            out_s[g % (2 * nh3)] = (hres[k] + y).astype(bf16)
            out_copy(g).start()
        return c

    with scope("phase3"):
        lax.fori_loop(0, ntrip, p3, 0)

    ng = S // t3
    with scope("waitend"):
        for g in range(ng - 2 * nh3, ng):
            out_copy(g).wait()


def make(sig=1, t1=512, t3=256, nh3=2, scopes=False, b1d=True):
    @jax.jit
    def fn(A_x, A_wqkv, A_wo, B_x, B_w1, B_b1, B_w2, B_b2):
        x = A_x.reshape(S, D)
        b1 = B_b1 if b1d else B_b1.reshape(1, F)
        b2 = B_b2 if b1d else B_b2.reshape(1, D)
        anyspec = pl.BlockSpec(memory_space=pl.ANY)
        vm = pl.BlockSpec(memory_space=pltpu.VMEM)
        out = pl.pallas_call(
            functools.partial(kernel, sig=sig, t1=t1, t3=t3, nh3=nh3, scopes=scopes),
            in_specs=[anyspec] * 7,
            out_specs=anyspec,
            out_shape=jax.ShapeDtypeStruct((S, D), bf16),
            scratch_shapes=[
                pltpu.VMEM((S, D), bf16),
                pltpu.VMEM((D, 3 * D), bf16),
                pltpu.VMEM((D, D), bf16),
                pltpu.VMEM((D, F), bf16),
                pltpu.VMEM((F, D), bf16),
                pltpu.VMEM((NTILE, S, 128), bf16),
                pltpu.VMEM((D, S), bf16),
                pltpu.VMEM((DV, S), f32),
                pltpu.VMEM((S, TQ), f32),
                pltpu.VMEM((S, TQ), f32),
                pltpu.VMEM((D, S), f32),
                pltpu.VMEM((2 * nh3, t3, D), bf16),
                pltpu.VMEM((F,), bf16),
                pltpu.VMEM((D,), bf16),
                pltpu.SemaphoreType.DMA((S // t1,)),
                pltpu.SemaphoreType.DMA((8,)),
                pltpu.SemaphoreType.DMA((2 * nh3,)),
            ],
            compiler_params=pltpu.CompilerParams(vmem_limit_bytes=100 * 1024 * 1024),
        )(x, A_wqkv, A_wo, B_w1, B_w2, b1, b2)
        return out.reshape(1, S, D)
    return fn


_fn = make()


@jax.jit
def pallas_sequential_preLN__softmax_full_mha__dense_activation_gelu__prompt_kernel(
    A_x: jax.Array,
    A_wqkv: jax.Array,
    A_wo: jax.Array,
    B_x: jax.Array,
    B_w1: jax.Array,
    B_b1: jax.Array,
    B_w2: jax.Array,
    B_b2: jax.Array,
):
    return _fn(A_x, A_wqkv, A_wo, B_x, B_w1, B_b1, B_w2, B_b2)
```

```python
import functools
import math
import jax
import jax.numpy as jnp
from jax import lax
import jax.experimental.pallas as pl
import jax.experimental.pallas.tpu as pltpu

S = 2048
D = 640
H = 32
DH = 20
F = 1536
NT5 = D // 128
NTILE = 9
VR = 24
DV = H * VR
TQ = 512
NQ = S // TQ
KC = 128
NSTEP = S // KC
EPS = 1e-5
QSCALE = (DH ** -0.5) * math.log2(math.e)
LMIN = 2.0 ** -80
MOFF = 40.0
ONES_LANE = (127, 127, 127, 127, 1, 65, 65, 65, 65)

TN = (((0,), (0,)), ((), ()))
f32 = jnp.float32
bf16 = jnp.bfloat16
u32 = jnp.uint32


def _ln(x):
    m = jnp.mean(x, axis=-1, keepdims=True)
    xc = x - m
    v = jnp.mean(xc * xc, axis=-1, keepdims=True)
    return xc * lax.rsqrt(v + EPS)


def _gelu(x):
    c = math.sqrt(2.0 / math.pi)
    return 0.5 * x * (1.0 + jnp.tanh(c * (x + 0.044715 * (x * x * x))))


class _Null:
    def __enter__(self):
        return self

    def __exit__(self, *a):
        return False


def kernel(x_hbm, wqkv_hbm, wo_hbm, w1_hbm, w2_hbm, b1_hbm, b2_hbm, o_hbm,
           x_s, wqkv_s, wo_s, w1_s, w2_s, k_s, qT_s, qTf_s, vT_s, sA, oT_s, out_s, b1_ref, b2_ref, cs_s,
           kb_all, kmx_s, zero_s, sem_x, sem_w, sem_o,
           *, t1, t3, nh3, scopes, ksplit, apc, lag, nch, pinset, pair, mpin, mergevq, slots7, slots8, apc0, pf32, over, zacc):
    over = dict(over)
    scope = jax.named_scope if scopes else (lambda name: _Null())
    n1 = S // t1
    spc = t1 // KC
    assist = list(apc0) + [t * spc + a for t in range(1, n1) for a in apc]
    grp_of = {c: g for g, c in enumerate(assist)}
    if pair:
        plist = [(g, None, j) for g in range(len(assist)) for j in range(TQ // 128)]
    else:
        plist = [(g, hf, j) for g in range(len(assist)) for hf in range(2) for j in range(TQ // 128)]
    halves = [(pc, k) for pc in plist for k in range(2)]
    work_at = {}
    _i = 0
    for _c in range(NSTEP):
        lst = []
        for (pos, w) in (over[_c] if _c in over else (slots7 if _c in grp_of else slots8)):
            take = halves[_i:_i + w]
            _i += len(take)
            for (pc, k) in take:
                assert assist[pc[0]] + lag - 2 >= _c >= assist[pc[0]] + lag - 14, (_c, pc)
                lst.append((pos, pc, k))
        work_at[_c] = lst
    assert _i == len(halves), (_i, len(halves))
    partial = {}
    tmask = [None]

    def rows_of(t, size):
        return pl.ds(t * size, size) if isinstance(t, int) else pl.ds(pl.multiple_of(t * size, size), size)

    def x_copy(t):
        rows = rows_of(t, t1)
        return pltpu.make_async_copy(x_hbm.at[rows, :], x_s.at[rows, :], sem_x.at[t])

    def wcols_copy(lo, n, sem):
        cols = pl.ds(lo, n)
        return pltpu.make_async_copy(wqkv_hbm.at[:, cols], wqkv_s.at[:, cols], sem_w.at[sem])

    wk1_copy = wcols_copy(D, ksplit, 0)
    wk2_copy = wcols_copy(D + ksplit, D - ksplit, 1)
    wv_copy = wcols_copy(2 * D, D, 2)
    wq_copy = wcols_copy(0, D, 3)
    wo_copy = pltpu.make_async_copy(wo_hbm, wo_s, sem_w.at[4])
    w1_copy = pltpu.make_async_copy(w1_hbm, w1_s, sem_w.at[5])
    w2_copy = pltpu.make_async_copy(w2_hbm, w2_s, sem_w.at[6])
    b1_copy = pltpu.make_async_copy(b1_hbm, b1_ref, sem_w.at[7])
    b2_copy = pltpu.make_async_copy(b2_hbm, b2_ref, sem_w.at[8])

    x_copy(0).start()
    wk1_copy.start()
    for _k in range(64):
        zero_s[_k] = 0

    def p1_mm(t, first, kmax):
        rows = rows_of(t, t1)
        xb = x_s[rows, :]
        xf = xb.astype(f32)
        mu = jnp.mean(xf, axis=-1, keepdims=True)
        xc = xf - mu
        r = lax.rsqrt(jnp.mean(xc * xc, axis=-1, keepdims=True) + EPS)
        if first:
            xb = jnp.concatenate([jnp.ones((16, D), bf16), xb], axis=0)

        def proj(lo, n, rr):
            cols = slice(lo, lo + n)
            y = jnp.dot(xb, wqkv_s[:, cols], preferred_element_type=f32)
            if first:
                c = y[0:1]
                cs_s[:, cols] = c
                y = y[16:]
            else:
                c = cs_s[:, cols]
            return (y - mu * c) * rr

        def kb_gen(krs, f0, f1):
            for ia, kr in enumerate(krs):
                g = ia if first else len(apc0) + (t - 1) * len(apc) + ia
                for f in range(f0, f1):
                    kb_all[g, f] = jnp.broadcast_to(kr[:, f:f + 1], (16, 128))

        if first:
            ya = proj(D, ksplit, r)
            wk2_copy.wait()
            y = jnp.concatenate([ya, proj(D + ksplit, D - ksplit, r)], axis=1)
        else:
            y = proj(D, D, r)
        ymax = jnp.max(jnp.abs(y).reshape(t1 // 8, 8, D), axis=0)
        kmax = ymax if kmax is None else jnp.maximum(kmax, ymax)
        lane = lax.broadcasted_iota(jnp.int32, (t1, 128), 1)
        hi = lane >= 64
        tiles = [y[:, 128 * j:128 * (j + 1)] for j in range(NT5)]
        for j in range(NT5):
            k_s[j, rows, :] = jnp.where(lane == ONES_LANE[j], 1.0, tiles[j]).astype(bf16)
        for j in range(NT5 - 1):
            seam = jnp.where(hi, tiles[j], tiles[j + 1])
            k_s[NT5 + j, rows, :] = jnp.where(lane == ONES_LANE[NT5 + j], 1.0, seam).astype(bf16)
        krs = [y[a * KC + KC - 16:a * KC + KC, :].astype(bf16).astype(f32) for a in (apc0 if first else apc)]
        if first:
            wv_copy.wait()
            if mergevq:
                wq_copy.wait()
                for tt in range(1, n1):
                    x_copy(tt).start()
            else:
                x_copy(1).start()
        kb_gen(krs, 0, D // 2)
        vT = proj(2 * D, D, r).astype(bf16).T.astype(f32)
        lo4 = lax.broadcasted_iota(jnp.int32, (8, t1), 0) < 4
        for p in range(H // 2):
            vT_s[48 * p:48 * p + 16, rows] = vT[40 * p:40 * p + 16]
            mid = vT[40 * p + 16:40 * p + 24]
            vT_s[48 * p + 16:48 * p + 24, rows] = jnp.where(lo4, mid, 1.0)
            vT_s[48 * p + 24:48 * p + 32, rows] = jnp.where(lo4, 1.0, mid)
            vT_s[48 * p + 32:48 * p + 48, rows] = vT[40 * p + 24:40 * p + 40]
        if first and not mergevq:
            wq_copy.wait()
            for tt in range(2, n1):
                x_copy(tt).start()
        kb_gen(krs, D // 2, D)
        qT = proj(0, D, r * QSCALE).astype(bf16).T
        qT_s[:, rows] = qT
        qTf_s[:, rows] = qT.astype(f32)
        return kmax

    def p1(t, kmax):
        x_copy(t).wait()
        return p1_mm(t, False, kmax)

    with scope("phase1"):
        wk2_copy.start()
        x_copy(0).wait()
        wk1_copy.wait()
        wv_copy.start()
        wq_copy.start()
        kmax0 = p1_mm(0, True, None)
        wo_copy.start()
        w1_copy.start()
        w2_copy.start()
        b1_copy.start()
        b2_copy.start()
        kmax = lax.fori_loop(1, n1, p1, kmax0)
        km = jnp.max(kmax, axis=0, keepdims=True) * (1.0 + 2.0 ** -7)
        kmx_s[...] = jnp.broadcast_to(km, (128, D)).T

    def dyn(v, m):
        return v if isinstance(v, int) else pl.multiple_of(v, m)

    def sel(c, a, b):
        return (a if c else b) if isinstance(c, bool) else jnp.where(c, a, b)

    def unit_m(pr, par, qb):
        rq = pl.ds(dyn(40 * pr + 16 * par, 8), VR)
        wf = qTf_s[rq, rows_of(qb, TQ)]
        kb = kmx_s[rq, :]
        prod = jnp.abs(wf) * jnp.concatenate([kb] * (TQ // 128), axis=1)
        r24 = lax.broadcasted_iota(jnp.int32, (VR, TQ), 0)
        valid = (r24 >= 4) if par else (r24 < DH)
        mneg = MOFF - jnp.sum(jnp.where(valid, prod, 0.0), axis=0, keepdims=True)
        return jnp.broadcast_to(mneg.astype(bf16).astype(f32), (8, TQ))

    def unit_q(pr, par, qb, mneg8):
        h = 2 * pr + par
        off = (h * DH) % 128
        t = (h * DH) // 128
        strad = off > 128 - DH
        tile = t + sel(strad, NT5, 0)
        olp = sel(strad, 32, sel(t == NT5 - 1, 0, 63))
        qcols = rows_of(qb, TQ)
        ra = pl.ds(dyn(128 * t + sel(strad, 128, 0), 64), 64)
        rb = pl.ds(dyn(128 * t + 64, 64), 64)
        w = jnp.concatenate([pltpu.bitcast(qT_s[ra, qcols], u32), pltpu.bitcast(qT_s[rb, qcols], u32)], axis=0)
        r = lax.broadcasted_iota(jnp.int32, (64, TQ), 0)
        msk = ((2 * r - off + 128) & 127) < DH
        if mneg8 is None:
            other = jnp.zeros((64, TQ), u32)
        else:
            mb = pltpu.bitcast(mneg8, u32)
            other = jnp.where(r == olp, jnp.concatenate([mb] * 8, axis=0), jnp.zeros((), u32))
        qm = pltpu.bitcast(jnp.where(msk, w, other), bf16)
        return qm, tile, (h, pr, par, qb, mneg8)

    def tree(terms):
        chains = [terms[k::nch] for k in range(nch)]
        sums = []
        for ch in chains:
            a = ch[0]
            for t_ in ch[1:]:
                a = a + t_
            sums.append(a)
        while len(sums) > 1:
            sums = [sums[k] + sums[k + 1] if k + 1 < len(sums) else sums[k] for k in range(0, len(sums), 2)]
        return sums[0]

    def vpu_half(info, pc, k):
        h, pr, par, qb, mneg8 = info
        g, hf, j = pc
        o4 = 4 * par
        rq2 = pl.ds(pl.multiple_of(40 * pr + 16 * par + zero_s[16 + (2 * g + hf) % 32] * 8, 8), VR)
        wf = qTf_s[rq2, pl.ds(qb * TQ + 128 * j, 128)]
        gz = g + zero_s[4 * qb + j]
        ds_ = range(DH // 2) if k == 0 else range(DH // 2, DH)
        terms = [kb_all[gz, h * DH + d, 8 * hf:8 * hf + 8, :] * wf[o4 + d:o4 + d + 1, :] for d in ds_]
        if k == 0:
            terms.append(mneg8[:, 128 * j:128 * (j + 1)])
        return terms

    def stepA(uq, c, extra_pin):
        qm, tile, info = uq
        nm = KC - 16 if c in grp_of else KC
        kk = k_s[tile, pl.ds(c * KC, nm), :]
        pins = []
        wk = work_at[c]
        i = 0
        while i < len(wk):
            pos, pc, k = wk[i]
            g, hf, j = pc
            dst = (pl.ds(assist[g] * KC + KC - 16 + 8 * hf, 8), slice(128 * j, 128 * (j + 1)))
            if k == 0 and i + 1 < len(wk) and wk[i + 1][0] == pos:
                v = tree(vpu_half(info, pc, 0) + vpu_half(info, pc, 1))
                sA[dst] = v
                i += 2
            elif k == 0:
                v = tree(vpu_half(info, pc, 0))
                sA[dst] = v
                i += 1
            else:
                v = tree(vpu_half(info, pc, 1) + [sA[dst]])
                sA[dst] = v
                i += 1
            pins.append((pos, v))
        pins += extra_pin
        pvpins = [v for pos, v in pins if pos == 9]
        pins = [(pos, v) for pos, v in pins if pos != 9]
        if pins:
            ku = pltpu.bitcast(kk, u32)
            parts = [ku[8 * j:8 * j + 8] for j in range(nm // 16)]
            for pos, v in pins:
                parts[pos] = jnp.where(tmask[0], parts[pos], pltpu.bitcast(v, u32))
            kk = pltpu.bitcast(jnp.concatenate(parts, axis=0), bf16)
        sA[pl.ds(c * KC, nm), :] = jnp.dot(kk, qm, preferred_element_type=f32)
        return pvpins

    def store_o(acc, pr, par, qb):
        orow = dyn(pr * 40, 8)
        qcols = rows_of(qb, TQ)
        if par == 0:
            l = acc[DH:DH + 1, :]
            oT_s[pl.ds(orow, VR), qcols] = acc * (1.0 / l)
        else:
            l = acc[0:1, :]
            o = acc * (1.0 / l)
            lo4 = lax.broadcasted_iota(jnp.int32, (8, TQ), 0) < 4
            mid_e = oT_s[pl.ds(orow + 16, 8), qcols]
            oT_s[pl.ds(orow + 16, 8), qcols] = jnp.where(lo4, mid_e, o[0:8])
            oT_s[pl.ds(orow + 24, 16), qcols] = o[8:24]
        return l

    def set_tmask():
        tmask[0] = (lax.broadcasted_iota(jnp.int32, (8, 128), 1) + zero_s[0]) >= 0

    with scope("prologue"):
        set_tmask()
        m0 = unit_m(0, 0, 0)
        uq = unit_q(0, 0, 0, m0)
        for c in range(lag):
            stepA(uq, c, [])

    def body(p, carry):
        lmin, m_cur = carry
        set_tmask()
        pn = jnp.minimum(p + 1, H // 2 - 1)
        acc = None
        uq = None
        ms = {0: m_cur}
        for n in range(8 * NSTEP):
            ka, ca = divmod(n + lag, NSTEP)
            if ca == 0 or n == 0:
                uq = unit_q(p if ka < 8 else pn, (ka % 8) // 4, ka % 4, ms[ka])
            extra = []
            if ca == mpin[0] and ka < 8:
                k2 = ka + 1
                ms[k2] = unit_m(p if k2 < 8 else pn, (k2 % 8) // 4, k2 % 4)
                extra = [(mpin[1], ms[k2][:, 128 * j:128 * (j + 1)]) for j in range(TQ // 128)]
            pvpins = stepA(uq, ca, extra)
            kb_, cb = divmod(n, NSTEP)
            par, qb = kb_ // 4, kb_ % 4
            vrow = pl.multiple_of(p * 48 + 24 * par, 8)
            pp = jnp.exp2(sA[pl.ds(cb * KC, KC), :])
            if not pf32:
                pp = pp.astype(bf16)
            vt = vT_s[pl.ds(vrow, VR), pl.ds(cb * KC, KC)]
            if pvpins:
                v0 = vt[0:8]
                for v in pvpins:
                    v0 = jnp.where(tmask[0], v0, v)
                vt = jnp.concatenate([v0, vt[8:]], axis=0)
            r = jnp.dot(vt, pp, preferred_element_type=f32)
            if cb == 0 and zacc:
                acc = jnp.full((VR, TQ), zero_s[1].astype(f32), f32) + r
            else:
                acc = r if cb == 0 else acc + r
            if cb == NSTEP - 1:
                l = store_o(acc, p, par, qb)
                lmin = jnp.minimum(lmin, jnp.where(l >= LMIN, 1.0, -1.0))
        return lmin, ms[8]

    with scope("attnloop"):
        lmin, _ = lax.fori_loop(0, H // 2, body, (jnp.ones((1, TQ), f32), m0))

    @pl.when(jnp.min(lmin) < 0.0)
    def _fallback():
        def unit(u, c0):
            pr = u // 8
            for par in range(2):
                @pl.when((u // 4) % 2 == par)
                def _():
                    qb = u % 4
                    qm, tile, _info = unit_q(pr, par, qb, None)

                    def pass1(c, m8):
                        krows = rows_of(c, KC)
                        s = jnp.dot(k_s[tile, krows, :], qm, preferred_element_type=f32)
                        sA[krows, :] = s
                        return jnp.maximum(m8, jnp.max(s.reshape(KC // 8, 8, TQ), axis=0))
                    m8 = lax.fori_loop(0, NSTEP, pass1, jnp.full((8, TQ), -jnp.inf, f32))
                    m = jnp.max(m8, axis=0, keepdims=True)
                    vrow = pl.multiple_of(pr * 48 + 24 * par, 8)

                    def pass2(c, acc):
                        krows = rows_of(c, KC)
                        pp = jnp.exp2(sA[krows, :] - m).astype(bf16)
                        return acc + jnp.dot(vT_s[pl.ds(vrow, VR), krows], pp, preferred_element_type=f32)
                    acc = lax.fori_loop(0, NSTEP, pass2, jnp.zeros((VR, TQ), f32))
                    store_o(acc, pr, par, qb)
            return c0
        lax.fori_loop(0, H * NQ, unit, 0)

    wo_copy.wait()
    w1_copy.wait()
    w2_copy.wait()
    b1_copy.wait()
    b2_copy.wait()

    ntrip = S // (t3 * nh3)

    def out_copy(g):
        slot = g % (2 * nh3)
        return pltpu.make_async_copy(out_s.at[slot], o_hbm.at[rows_of(g, t3), :], sem_o.at[slot])

    def p3(trip, c):
        @pl.when(trip >= 2)
        def _():
            for k in range(nh3):
                out_copy((trip - 2) * nh3 + k).wait()

        b1 = b1_ref[...].reshape(1, F).astype(f32)
        b2 = b2_ref[...].reshape(1, D).astype(f32)
        hres = []
        for k in range(nh3):
            rows = rows_of(trip * nh3 + k, t3)
            oT = oT_s[:, rows].astype(bf16)
            attn = lax.dot_general(oT, wo_s[...], TN, preferred_element_type=f32)
            hres.append(x_s[rows, :].astype(f32) + attn)
        act = []
        for k in range(nh3):
            hn = _ln(hres[k]).astype(bf16)
            a = jnp.dot(hn, w1_s[...], preferred_element_type=f32) + b1
            act.append(_gelu(a).astype(bf16))
        for k in range(nh3):
            g = trip * nh3 + k
            y = jnp.dot(act[k], w2_s[...], preferred_element_type=f32) + b2
            out_s[g % (2 * nh3)] = (hres[k] + y).astype(bf16)
            out_copy(g).start()
        return c

    with scope("phase3"):
        lax.fori_loop(0, ntrip, p3, 0)

    ng = S // t3
    with scope("waitend"):
        for g in range(ng - 2 * nh3, ng):
            out_copy(g).wait()


def make(t1=512, t3=256, nh3=2, scopes=False, ksplit=256, apc=(1, 3), lag=4, nch=4, pinset=(2, 3, 4, 5, 6),
         pair=False, mpin=(10, 1), mergevq=True, slots7=((3, 2), (4, 2), (5, 2), (6, 2)), slots8=((3, 2), (4, 2), (5, 2), (6, 2)), apc0=(1, 3), pf32=False, over=(), zacc=True):
    ngrp = max(len(apc0) + len(apc) * (S // t1 - 1), 1)

    @jax.jit
    def fn(A_x, A_wqkv, A_wo, B_x, B_w1, B_b1, B_w2, B_b2):
        x = A_x.reshape(S, D)
        anyspec = pl.BlockSpec(memory_space=pl.ANY)
        out = pl.pallas_call(
            functools.partial(kernel, t1=t1, t3=t3, nh3=nh3, scopes=scopes, ksplit=ksplit, apc=tuple(apc),
                              lag=lag, nch=nch, pinset=tuple(pinset), pair=pair, mpin=tuple(mpin), mergevq=mergevq, slots7=slots7, slots8=slots8, apc0=tuple(apc0), pf32=pf32, over=over, zacc=zacc),
            in_specs=[anyspec] * 7,
            out_specs=anyspec,
            out_shape=jax.ShapeDtypeStruct((S, D), bf16),
            scratch_shapes=[
                pltpu.VMEM((S, D), bf16),
                pltpu.VMEM((D, 3 * D), bf16),
                pltpu.VMEM((D, D), bf16),
                pltpu.VMEM((D, F), bf16),
                pltpu.VMEM((F, D), bf16),
                pltpu.VMEM((NTILE, S, 128), bf16),
                pltpu.VMEM((D, S), bf16),
                pltpu.VMEM((D, S), f32),
                pltpu.VMEM((DV, S), f32),
                pltpu.VMEM((S, TQ), f32),
                pltpu.VMEM((D, S), f32),
                pltpu.VMEM((2 * nh3, t3, D), bf16),
                pltpu.VMEM((F,), bf16),
                pltpu.VMEM((D,), bf16),
                pltpu.VMEM((1, 2944), f32),
                pltpu.VMEM((ngrp, D, 16, 128), f32),
                pltpu.VMEM((D, 128), f32),
                pltpu.SMEM((64,), jnp.int32),
                pltpu.SemaphoreType.DMA((S // t1,)),
                pltpu.SemaphoreType.DMA((9,)),
                pltpu.SemaphoreType.DMA((2 * nh3,)),
            ],
            compiler_params=pltpu.CompilerParams(vmem_limit_bytes=110 * 1024 * 1024),
        )(x, A_wqkv, A_wo, B_w1, B_w2, B_b1, B_b2)
        return out.reshape(1, S, D)
    return fn


_fn = make(apc0=(2,3), apc=(1,2,3), slots7=((0,1),(1,1),(2,1),(3,2),(4,2),(5,2),(6,2),(9,1)), slots8=((0,1),(1,1),(2,1),(3,2),(4,2),(5,2),(6,2),(7,2),(9,1)), over=((4,((3,2),(4,2),(5,2),(6,2))),(5,((5,2),(6,2)))), mpin=(10,9))


@jax.jit
def pallas_sequential_preLN__softmax_full_mha__dense_activation_gelu__prompt_kernel(
    A_x: jax.Array,
    A_wqkv: jax.Array,
    A_wo: jax.Array,
    B_x: jax.Array,
    B_w1: jax.Array,
    B_b1: jax.Array,
    B_w2: jax.Array,
    B_b2: jax.Array,
):
    return _fn(A_x, A_wqkv, A_wo, B_x, B_w1, B_b1, B_w2, B_b2)
```

```python
import functools
import math
import jax
import jax.numpy as jnp
from jax import lax
import jax.experimental.pallas as pl
import jax.experimental.pallas.tpu as pltpu

S = 2048
D = 640
H = 32
DH = 20
F = 1536
NT5 = D // 128
NTILE = 9
VR = 24
DV = H * VR
TQ = 512
NQ = S // TQ
KC = 128
NSTEP = S // KC
EPS = 1e-5
QSCALE = (DH ** -0.5) * math.log2(math.e)
LMIN = 2.0 ** -80
MOFF = 40.0
AMAX = 2.0 ** 120
ONES_LANE = (127, 127, 127, 127, 1, 65, 65, 65, 65)

TN = (((0,), (0,)), ((), ()))
f32 = jnp.float32
bf16 = jnp.bfloat16
u32 = jnp.uint32


def _ln(x):
    m = jnp.mean(x, axis=-1, keepdims=True)
    xc = x - m
    v = jnp.mean(xc * xc, axis=-1, keepdims=True)
    return xc * lax.rsqrt(v + EPS)


def _gelu(x):
    c = math.sqrt(2.0 / math.pi)
    return 0.5 * x * (1.0 + jnp.tanh(c * (x + 0.044715 * (x * x * x))))


class _Null:
    def __enter__(self):
        return self

    def __exit__(self, *a):
        return False


def kernel(x_hbm, wqkv_hbm, wo_hbm, w1_hbm, w2_hbm, b1_hbm, b2_hbm, o_hbm,
           x_s, wqkv_s, wo_s, w1_s, w2_s, k_s, qT_s, qTf_s, vT_s, sA, oT_s, out_s, b1_ref, b2_ref, cs_s,
           kb_all, kmx_s, zero_s, sem_x, sem_w, sem_o,
           *, t1, t3, nh3, scopes, ksplit, apc, lag, nch, pinset, pair, mpin, mergevq, slots7, slots8, apc0, pf32, over, zacc, frcp, fchk):
    over = dict(over)
    scope = jax.named_scope if scopes else (lambda name: _Null())
    n1 = S // t1
    spc = t1 // KC
    assist = list(apc0) + [t * spc + a for t in range(1, n1) for a in apc]
    grp_of = {c: g for g, c in enumerate(assist)}
    quanta = [(g, j, k) for g in range(len(assist)) for j in range(TQ // 128) for k in range(4)]
    work_at = {}
    _i = 0
    for _c in range(NSTEP):
        lst = []
        for (pos, w) in (over[_c] if _c in over else (slots7 if _c in grp_of else slots8)):
            take = quanta[_i:_i + w]
            _i += len(take)
            for qn in take:
                assert assist[qn[0]] + lag - 2 >= _c >= assist[qn[0]] + lag - 14, (_c, qn)
                lst.append((pos, qn))
        work_at[_c] = lst
    assert _i == len(quanta), (_i, len(quanta))
    tmask = [None]

    def rows_of(t, size):
        return pl.ds(t * size, size) if isinstance(t, int) else pl.ds(pl.multiple_of(t * size, size), size)

    def x_copy(t):
        rows = rows_of(t, t1)
        return pltpu.make_async_copy(x_hbm.at[rows, :], x_s.at[rows, :], sem_x.at[t])

    def wcols_copy(lo, n, sem):
        cols = pl.ds(lo, n)
        return pltpu.make_async_copy(wqkv_hbm.at[:, cols], wqkv_s.at[:, cols], sem_w.at[sem])

    wk1_copy = wcols_copy(D, ksplit, 0)
    wk2_copy = wcols_copy(D + ksplit, D - ksplit, 1)
    wv_copy = wcols_copy(2 * D, D, 2)
    wq_copy = wcols_copy(0, D, 3)
    wo_copy = pltpu.make_async_copy(wo_hbm, wo_s, sem_w.at[4])
    w1_copy = pltpu.make_async_copy(w1_hbm, w1_s, sem_w.at[5])
    w2_copy = pltpu.make_async_copy(w2_hbm, w2_s, sem_w.at[6])
    b1_copy = pltpu.make_async_copy(b1_hbm, b1_ref, sem_w.at[7])
    b2_copy = pltpu.make_async_copy(b2_hbm, b2_ref, sem_w.at[8])

    x_copy(0).start()
    wk1_copy.start()
    for _k in range(64):
        zero_s[_k] = 0

    def p1_mm(t, first, kmax):
        rows = rows_of(t, t1)
        rows2 = rows_of(t, t1 // 2)
        xb = x_s[rows, :]
        xf = xb.astype(f32)
        mu = jnp.mean(xf, axis=-1, keepdims=True)
        xc = xf - mu
        r = lax.rsqrt(jnp.mean(xc * xc, axis=-1, keepdims=True) + EPS)
        if first:
            xb = jnp.concatenate([jnp.ones((16, D), bf16), xb], axis=0)

        def proj(lo, n, rr):
            cols = slice(lo, lo + n)
            y = jnp.dot(xb, wqkv_s[:, cols], preferred_element_type=f32)
            if first:
                c = y[0:1]
                cs_s[:, cols] = c
                y = y[16:]
            else:
                c = cs_s[:, cols]
            return (y - mu * c) * rr

        def kb_gen(krs, f0, f1):
            if not krs:
                return
            g0 = 0 if first else len(apc0) + (t - 1) * len(apc)
            kr = jnp.concatenate(krs, axis=0)
            for f in range(f0, f1):
                bc = jnp.broadcast_to(kr[:, f:f + 1], (16 * len(krs), 128))
                for ia in range(len(krs)):
                    kb_all[g0 + ia, f] = bc[16 * ia:16 * ia + 16]

        if first:
            ya = proj(D, ksplit, r)
            wk2_copy.wait()
            y = jnp.concatenate([ya, proj(D + ksplit, D - ksplit, r)], axis=1)
        else:
            y = proj(D, D, r)
        ymax = jnp.max(jnp.abs(y).reshape(t1 // 8, 8, D), axis=0)
        kmax = ymax if kmax is None else jnp.maximum(kmax, ymax)
        lane = lax.broadcasted_iota(jnp.int32, (t1, 128), 1)
        hi = lane >= 64
        tiles = [y[:, 128 * j:128 * (j + 1)] for j in range(NT5)]
        for j in range(NT5):
            k_s[j, rows2, :] = pltpu.bitcast(jnp.where(lane == ONES_LANE[j], 1.0, tiles[j]).astype(bf16), u32)
        for j in range(NT5 - 1):
            seam = jnp.where(hi, tiles[j], tiles[j + 1])
            k_s[NT5 + j, rows2, :] = pltpu.bitcast(jnp.where(lane == ONES_LANE[NT5 + j], 1.0, seam).astype(bf16), u32)
        krs = [y[a * KC + KC - 16:a * KC + KC, :].astype(bf16).astype(f32) for a in (apc0 if first else apc)]
        if first:
            wv_copy.wait()
            if mergevq:
                wq_copy.wait()
                for tt in range(1, n1):
                    x_copy(tt).start()
            else:
                x_copy(1).start()
        kb_gen(krs, 0, D // 2)
        vT = proj(2 * D, D, r).astype(bf16).T.astype(f32)
        lo4 = lax.broadcasted_iota(jnp.int32, (8, t1), 0) < 4
        for p in range(H // 2):
            vT_s[48 * p:48 * p + 16, rows] = vT[40 * p:40 * p + 16]
            mid = vT[40 * p + 16:40 * p + 24]
            vT_s[48 * p + 16:48 * p + 24, rows] = jnp.where(lo4, mid, 1.0)
            vT_s[48 * p + 24:48 * p + 32, rows] = jnp.where(lo4, 1.0, mid)
            vT_s[48 * p + 32:48 * p + 48, rows] = vT[40 * p + 24:40 * p + 40]
        if first and not mergevq:
            wq_copy.wait()
            for tt in range(2, n1):
                x_copy(tt).start()
        kb_gen(krs, D // 2, D)
        qT = proj(0, D, r * QSCALE).astype(bf16).T
        qT_s[:, rows] = pltpu.bitcast(qT, u32)
        qTf_s[:, rows] = qT.astype(f32)
        return kmax

    def p1(t, kmax):
        x_copy(t).wait()
        return p1_mm(t, False, kmax)

    with scope("phase1"):
        wk2_copy.start()
        x_copy(0).wait()
        wk1_copy.wait()
        wv_copy.start()
        wq_copy.start()
        kmax0 = p1_mm(0, True, None)
        wo_copy.start()
        w1_copy.start()
        w2_copy.start()
        b1_copy.start()
        b2_copy.start()
        kmax = lax.fori_loop(1, n1, p1, kmax0)
        km = jnp.max(kmax, axis=0, keepdims=True) * (1.0 + 2.0 ** -7)
        kmx_s[...] = jnp.broadcast_to(km, (128, D)).T

    def dyn(v, m):
        return v if isinstance(v, int) else pl.multiple_of(v, m)

    def sel(c, a, b):
        return (a if c else b) if isinstance(c, bool) else jnp.where(c, a, b)

    def unit_m(pr, par, qb):
        rq = pl.ds(dyn(40 * pr + 16 * par, 8), VR)
        wf = qTf_s[rq, rows_of(qb, TQ)]
        kb = kmx_s[rq, :]
        prod = jnp.abs(wf) * jnp.concatenate([kb] * (TQ // 128), axis=1)
        r24 = lax.broadcasted_iota(jnp.int32, (VR, TQ), 0)
        valid = (r24 >= 4) if par else (r24 < DH)
        mneg = MOFF - jnp.sum(jnp.where(valid, prod, 0.0), axis=0, keepdims=True)
        return jnp.broadcast_to(mneg.astype(bf16).astype(f32), (8, TQ))

    def unit_q(pr, par, qb, mneg8):
        h = 2 * pr + par
        off = (h * DH) % 128
        t = (h * DH) // 128
        strad = off > 128 - DH
        tile = t + sel(strad, NT5, 0)
        olp = sel(strad, 32, sel(t == NT5 - 1, 0, 63))
        qcols = rows_of(qb, TQ)
        ra = pl.ds(dyn(64 * t + sel(strad, 64, 0), 32), 32)
        rb = pl.ds(dyn(64 * t + 32, 32), 32)
        w = jnp.concatenate([qT_s[ra, qcols], qT_s[rb, qcols]], axis=0)
        r = lax.broadcasted_iota(jnp.int32, (64, TQ), 0)
        msk = ((2 * r - off + 128) & 127) < DH
        if mneg8 is None:
            other = jnp.zeros((64, TQ), u32)
        else:
            mb = pltpu.bitcast(mneg8, u32)
            other = jnp.where(r == olp, jnp.concatenate([mb] * 8, axis=0), jnp.zeros((), u32))
        qm = pltpu.bitcast(jnp.where(msk, w, other), bf16)
        return qm, tile, (h, pr, par, qb, mneg8)

    def tree(terms):
        chains = [terms[k::nch] for k in range(min(nch, len(terms)))]
        sums = []
        for ch in chains:
            a = ch[0]
            for t_ in ch[1:]:
                a = a + t_
            sums.append(a)
        while len(sums) > 1:
            sums = [sums[k] + sums[k + 1] if k + 1 < len(sums) else sums[k] for k in range(0, len(sums), 2)]
        return sums[0]

    def vpu_terms(info, qn):
        h, pr, par, qb, mneg8 = info
        g, j, k = qn
        o4 = 4 * par
        rq2 = pl.ds(pl.multiple_of(40 * pr + 16 * par + zero_s[16 + g] * 8, 8), VR)
        wf = qTf_s[rq2, pl.ds(qb * TQ + 128 * j, 128)]
        gz = g + zero_s[4 * qb + j]
        terms = [kb_all[gz, h * DH + d].reshape(2, 8, 128) * wf[o4 + d:o4 + d + 1, :][None]
                 for d in range(5 * k, 5 * k + 5)]
        if k == 0:
            terms.append(jnp.broadcast_to(mneg8[None, :, 128 * j:128 * (j + 1)], (2, 8, 128)))
        return terms

    def stepA(uq, c, extra_pin):
        qm, tile, info = uq
        nm = KC - 16 if c in grp_of else KC
        ku = k_s[tile, pl.ds(c * KC // 2, nm // 2), :]
        pins = []
        wk = work_at[c]
        i = 0
        while i < len(wk):
            pos, qn = wk[i]
            g, j, k = qn
            dst = (pl.ds(assist[g] * KC + KC - 16, 16), slice(128 * j, 128 * (j + 1)))
            terms = vpu_terms(info, qn)
            i += 1
            while i < len(wk) and wk[i][0] == pos and wk[i][1][:2] == (g, j):
                terms += vpu_terms(info, wk[i][1])
                i += 1
            if k > 0:
                terms.append(sA[dst].reshape(2, 8, 128))
            v = tree(terms)
            sA[dst] = v.reshape(16, 128)
            pins.append((pos, v[0]))
            pins.append((pos, v[1]))
        pins += extra_pin
        pvpins = [v for pos, v in pins if pos == 9]
        pins = [(pos, v) for pos, v in pins if pos != 9]
        kk = pltpu.bitcast(ku, bf16)
        if pins:
            parts = [ku[8 * j:8 * j + 8] for j in range(nm // 16)]
            for pos, v in pins:
                parts[pos] = jnp.where(tmask[0], parts[pos], pltpu.bitcast(v, u32))
            kk = pltpu.bitcast(jnp.concatenate(parts, axis=0), bf16)
        sA[pl.ds(c * KC, nm), :] = jnp.dot(kk, qm, preferred_element_type=f32)
        return pvpins

    def recip(l, fast):
        if not fast:
            return 1.0 / l
        y = pl.reciprocal(l, approx=True)
        y = y * (2.0 - l * y)
        return y * (2.0 - l * y)

    def store_o(acc, pr, par, qb, fast=False):
        orow = dyn(pr * 40, 8)
        qcols = rows_of(qb, TQ)
        if par == 0:
            l = acc[DH:DH + 1, :]
            oT_s[pl.ds(orow, VR), qcols] = acc * recip(l, fast)
        else:
            l = acc[0:1, :]
            o = acc * recip(l, fast)
            lo4 = lax.broadcasted_iota(jnp.int32, (8, TQ), 0) < 4
            mid_e = oT_s[pl.ds(orow + 16, 8), qcols]
            oT_s[pl.ds(orow + 16, 8), qcols] = jnp.where(lo4, mid_e, o[0:8])
            oT_s[pl.ds(orow + 24, 16), qcols] = o[8:24]
        return l

    def set_tmask():
        tmask[0] = (lax.broadcasted_iota(jnp.int32, (8, 128), 1) + zero_s[0]) >= 0

    with scope("prologue"):
        set_tmask()
        m0 = unit_m(0, 0, 0)
        uq = unit_q(0, 0, 0, m0)
        for c in range(lag):
            stepA(uq, c, [])

    def body(p, carry):
        lmin, m_cur = carry
        set_tmask()
        pn = jnp.minimum(p + 1, H // 2 - 1)
        acc = None
        uq = None
        ms = {0: m_cur}
        for n in range(8 * NSTEP):
            ka, ca = divmod(n + lag, NSTEP)
            if ca == 0 or n == 0:
                uq = unit_q(p if ka < 8 else pn, (ka % 8) // 4, ka % 4, ms[ka])
            extra = []
            if ca == mpin[0] and ka < 8:
                k2 = ka + 1
                ms[k2] = unit_m(p if k2 < 8 else pn, (k2 % 8) // 4, k2 % 4)
                extra = [(mpin[1], ms[k2][:, 128 * j:128 * (j + 1)]) for j in range(TQ // 128)]
            pvpins = stepA(uq, ca, extra)
            kb_, cb = divmod(n, NSTEP)
            par, qb = kb_ // 4, kb_ % 4
            vrow = pl.multiple_of(p * 48 + 24 * par, 8)
            pp = jnp.exp2(sA[pl.ds(cb * KC, KC), :])
            if not pf32:
                pp = pp.astype(bf16)
            vt = vT_s[pl.ds(vrow, VR), pl.ds(cb * KC, KC)]
            if pvpins:
                v0 = vt[0:8]
                for v in pvpins:
                    v0 = jnp.where(tmask[0], v0, v)
                vt = jnp.concatenate([v0, vt[8:]], axis=0)
            r = jnp.dot(vt, pp, preferred_element_type=f32)
            if cb == 0 and zacc:
                acc = jnp.full((VR, TQ), zero_s[1].astype(f32), f32) + r
            else:
                acc = r if cb == 0 else acc + r
            if cb == NSTEP - 1:
                l = store_o(acc, p, par, qb, frcp)
                if fchk:
                    aa = jnp.abs(acc)
                    big = jnp.maximum(jnp.maximum(aa[0:8], aa[8:16]), aa[16:24])
                    good = jnp.logical_and(big <= AMAX, l >= LMIN)
                    lmin = jnp.minimum(lmin, jnp.where(good, 1.0, -1.0))
                else:
                    lmin = jnp.minimum(lmin, jnp.where(l >= LMIN, 1.0, -1.0))
        return lmin, ms[8]

    with scope("attnloop"):
        lmin, _ = lax.fori_loop(0, H // 2, body, (jnp.ones((8 if fchk else 1, TQ), f32), m0))

    @pl.when(jnp.min(lmin) < 0.0)
    def _fallback():
        def unit(u, c0):
            pr = u // 8
            for par in range(2):
                @pl.when((u // 4) % 2 == par)
                def _():
                    qb = u % 4
                    qm, tile, _info = unit_q(pr, par, qb, None)

                    def pass1(c, m8):
                        krows = rows_of(c, KC)
                        s = jnp.dot(pltpu.bitcast(k_s[tile, rows_of(c, KC // 2), :], bf16), qm, preferred_element_type=f32)
                        sA[krows, :] = s
                        return jnp.maximum(m8, jnp.max(s.reshape(KC // 8, 8, TQ), axis=0))
                    m8 = lax.fori_loop(0, NSTEP, pass1, jnp.full((8, TQ), -jnp.inf, f32))
                    m = jnp.max(m8, axis=0, keepdims=True)
                    vrow = pl.multiple_of(pr * 48 + 24 * par, 8)

                    def pass2(c, acc):
                        krows = rows_of(c, KC)
                        pp = jnp.exp2(sA[krows, :] - m).astype(bf16)
                        return acc + jnp.dot(vT_s[pl.ds(vrow, VR), krows], pp, preferred_element_type=f32)
                    acc = lax.fori_loop(0, NSTEP, pass2, jnp.zeros((VR, TQ), f32))
                    store_o(acc, pr, par, qb)
            return c0
        lax.fori_loop(0, H * NQ, unit, 0)

    wo_copy.wait()
    w1_copy.wait()
    w2_copy.wait()
    b1_copy.wait()
    b2_copy.wait()

    ntrip = S // (t3 * nh3)

    def out_copy(g):
        slot = g % (2 * nh3)
        return pltpu.make_async_copy(out_s.at[slot], o_hbm.at[rows_of(g, t3), :], sem_o.at[slot])

    def p3(trip, c):
        @pl.when(trip >= 2)
        def _():
            for k in range(nh3):
                out_copy((trip - 2) * nh3 + k).wait()

        b1 = b1_ref[...].reshape(1, F).astype(f32)
        b2 = b2_ref[...].reshape(1, D).astype(f32)
        hres = []
        for k in range(nh3):
            rows = rows_of(trip * nh3 + k, t3)
            oT = oT_s[:, rows].astype(bf16)
            attn = lax.dot_general(oT, wo_s[...], TN, preferred_element_type=f32)
            hres.append(x_s[rows, :].astype(f32) + attn)
        act = []
        for k in range(nh3):
            hn = _ln(hres[k]).astype(bf16)
            a = jnp.dot(hn, w1_s[...], preferred_element_type=f32) + b1
            act.append(_gelu(a).astype(bf16))
        for k in range(nh3):
            g = trip * nh3 + k
            y = jnp.dot(act[k], w2_s[...], preferred_element_type=f32) + b2
            out_s[g % (2 * nh3)] = (hres[k] + y).astype(bf16)
            out_copy(g).start()
        return c

    with scope("phase3"):
        lax.fori_loop(0, ntrip, p3, 0)

    ng = S // t3
    with scope("waitend"):
        for g in range(ng - 2 * nh3, ng):
            out_copy(g).wait()


def make(t1=512, t3=256, nh3=2, scopes=False, ksplit=256, apc=(1, 2, 3), lag=4, nch=3, pinset=(2, 3, 4, 5, 6),
         pair=False, mpin=(10, 9), mergevq=True, slots7=((0,1),(1,1),(2,2),(3,2),(4,2),(5,2),(6,2),(9,1)), slots8=((0,1),(1,1),(2,2),(3,2),(4,2),(5,2),(6,2),(7,2),(9,1)), apc0=(1, 2, 3), pf32=False, over=((4,((3,2),(4,2),(5,2),(6,2))),(5,((5,2),(6,2)))), zacc=True, frcp=False, fchk=True, vmem=116):
    ngrp = max(len(apc0) + len(apc) * (S // t1 - 1), 1)

    @jax.jit
    def fn(A_x, A_wqkv, A_wo, B_x, B_w1, B_b1, B_w2, B_b2):
        x = A_x.reshape(S, D)
        anyspec = pl.BlockSpec(memory_space=pl.ANY)
        out = pl.pallas_call(
            functools.partial(kernel, t1=t1, t3=t3, nh3=nh3, scopes=scopes, ksplit=ksplit, apc=tuple(apc),
                              lag=lag, nch=nch, pinset=tuple(pinset), pair=pair, mpin=tuple(mpin), mergevq=mergevq, slots7=slots7, slots8=slots8, apc0=tuple(apc0), pf32=pf32, over=over, zacc=zacc, frcp=frcp, fchk=fchk),
            in_specs=[anyspec] * 7,
            out_specs=anyspec,
            out_shape=jax.ShapeDtypeStruct((S, D), bf16),
            scratch_shapes=[
                pltpu.VMEM((S, D), bf16),
                pltpu.VMEM((D, 3 * D), bf16),
                pltpu.VMEM((D, D), bf16),
                pltpu.VMEM((D, F), bf16),
                pltpu.VMEM((F, D), bf16),
                pltpu.VMEM((NTILE, S // 2, 128), u32),
                pltpu.VMEM((D // 2, S), u32),
                pltpu.VMEM((D, S), f32),
                pltpu.VMEM((DV, S), f32),
                pltpu.VMEM((S, TQ), f32),
                pltpu.VMEM((D, S), f32),
                pltpu.VMEM((2 * nh3, t3, D), bf16),
                pltpu.VMEM((F,), bf16),
                pltpu.VMEM((D,), bf16),
                pltpu.VMEM((1, 2944), f32),
                pltpu.VMEM((ngrp, D, 16, 128), f32),
                pltpu.VMEM((D, 128), f32),
                pltpu.SMEM((64,), jnp.int32),
                pltpu.SemaphoreType.DMA((S // t1,)),
                pltpu.SemaphoreType.DMA((9,)),
                pltpu.SemaphoreType.DMA((2 * nh3,)),
            ],
            compiler_params=pltpu.CompilerParams(vmem_limit_bytes=vmem * 1024 * 1024),
        )(x, A_wqkv, A_wo, B_w1, B_w2, B_b1, B_b2)
        return out.reshape(1, S, D)
    return fn


_fn = make()


@jax.jit
def pallas_sequential_preLN__softmax_full_mha__dense_activation_gelu__prompt_kernel(
    A_x: jax.Array,
    A_wqkv: jax.Array,
    A_wo: jax.Array,
    B_x: jax.Array,
    B_w1: jax.Array,
    B_b1: jax.Array,
    B_w2: jax.Array,
    B_b2: jax.Array,
):
    return _fn(A_x, A_wqkv, A_wo, B_x, B_w1, B_b1, B_w2, B_b2)
```

```python
import functools
import math

import jax
import jax.numpy as jnp
from jax import lax
import jax.experimental.pallas as pl
import jax.experimental.pallas.tpu as pltpu

S = 2048
D = 640
H = 32
DH = 20
F = 1536
NT5 = D // 128
NTILE = 9
VR = 24
DV = H * VR
TQ = 512
NQ = S // TQ
KC = 128
NSTEP = S // KC
EPS = 1e-5
QSCALE = (DH ** -0.5) * math.log2(math.e)
MOFF = 40.0
LMIN = 2.0 ** -80
AMAX = 2.0 ** 120
ONES_LANE = (127, 127, 127, 127, 1, 65, 65, 65, 65)

T1 = 512
N1 = S // T1
KSPLIT = 256
T3 = 256
NH3 = 2
LAG = 4
APC = (1, 2, 3)
ASSIST = tuple(t * (T1 // KC) + a for t in range(N1) for a in APC)
NGRP = len(ASSIST)
SLOTS7 = ((0, 1), (1, 1), (2, 2), (3, 2), (4, 2), (5, 2), (6, 2), (9, 1))
SLOTS8 = ((0, 1), (1, 1), (2, 2), (3, 2), (4, 2), (5, 2), (6, 2), (7, 2), (9, 1))
SLOTS_AT = {4: ((3, 2), (4, 2), (5, 2), (6, 2)), 5: ((5, 2), (6, 2))}
MSTEP = 10
NCH = 2

TN = (((0,), (0,)), ((), ()))
f32 = jnp.float32
bf16 = jnp.bfloat16
u32 = jnp.uint32


def _plan_vpu_work():
    quanta = [(g, j, k) for g in range(NGRP) for j in range(TQ // 128) for k in range(4)]
    work_at = {}
    i = 0
    for c in range(NSTEP):
        lst = []
        for pos, w in SLOTS_AT.get(c, SLOTS7 if c in ASSIST else SLOTS8):
            take = quanta[i:i + w]
            i += len(take)
            for qn in take:
                assert ASSIST[qn[0]] + LAG - 2 >= c >= ASSIST[qn[0]] + LAG - 14
                lst.append((pos, qn))
        work_at[c] = lst
    assert i == len(quanta)
    return work_at


WORK_AT = _plan_vpu_work()


def _ln(x):
    m = jnp.mean(x, axis=-1, keepdims=True)
    xc = x - m
    v = jnp.mean(xc * xc, axis=-1, keepdims=True)
    return xc * lax.rsqrt(v + EPS)


def _gelu(x):
    c = math.sqrt(2.0 / math.pi)
    return 0.5 * x * (1.0 + jnp.tanh(c * (x + 0.044715 * (x * x * x))))


def _rows(t, size):
    return pl.ds(t * size, size) if isinstance(t, int) else pl.ds(pl.multiple_of(t * size, size), size)


def _dyn(v, m):
    return v if isinstance(v, int) else pl.multiple_of(v, m)


def _sel(c, a, b):
    return (a if c else b) if isinstance(c, bool) else jnp.where(c, a, b)


def _kernel(x_hbm, wqkv_hbm, wo_hbm, w1_hbm, w2_hbm, b1_hbm, b2_hbm, o_hbm,
            x_s, wqkv_s, wo_s, w1_s, w2_s, k_s, qT_s, qTf_s, vT_s, sA, oT_s, out_s, b1_ref, b2_ref, cs_s,
            kb_all, kmx_s, zero_s, sem_x, sem_w, sem_o):

    def x_copy(t):
        rows = _rows(t, T1)
        return pltpu.make_async_copy(x_hbm.at[rows, :], x_s.at[rows, :], sem_x.at[t])

    def wcols_copy(lo, n, sem):
        cols = pl.ds(lo, n)
        return pltpu.make_async_copy(wqkv_hbm.at[:, cols], wqkv_s.at[:, cols], sem_w.at[sem])

    wk1_copy = wcols_copy(D, KSPLIT, 0)
    wk2_copy = wcols_copy(D + KSPLIT, D - KSPLIT, 1)
    wv_copy = wcols_copy(2 * D, D, 2)
    wq_copy = wcols_copy(0, D, 3)
    wo_copy = pltpu.make_async_copy(wo_hbm, wo_s, sem_w.at[4])
    w1_copy = pltpu.make_async_copy(w1_hbm, w1_s, sem_w.at[5])
    w2_copy = pltpu.make_async_copy(w2_hbm, w2_s, sem_w.at[6])
    b1_copy = pltpu.make_async_copy(b1_hbm, b1_ref, sem_w.at[7])
    b2_copy = pltpu.make_async_copy(b2_hbm, b2_ref, sem_w.at[8])

    x_copy(0).start()
    wk1_copy.start()
    for k in range(64):
        zero_s[k] = 0

    def p1_chunk(t, first, kmax):
        rows = _rows(t, T1)
        rows2 = _rows(t, T1 // 2)
        xb = x_s[rows, :]
        xf = xb.astype(f32)
        mu = jnp.mean(xf, axis=-1, keepdims=True)
        xc = xf - mu
        r = lax.rsqrt(jnp.mean(xc * xc, axis=-1, keepdims=True) + EPS)
        if first:
            xb = jnp.concatenate([jnp.ones((16, D), bf16), xb], axis=0)

        def proj(lo, n, rr):
            cols = slice(lo, lo + n)
            y = jnp.dot(xb, wqkv_s[:, cols], preferred_element_type=f32)
            if first:
                c = y[0:1]
                cs_s[:, cols] = c
                y = y[16:]
            else:
                c = cs_s[:, cols]
            return (y - mu * c) * rr

        def kb_gen(krs, f0, f1):
            g0 = t * len(APC)
            kr = jnp.concatenate(krs, axis=0)
            for f in range(f0, f1):
                bc = jnp.broadcast_to(kr[:, f:f + 1], (16 * len(krs), 128))
                for ia in range(len(krs)):
                    kb_all[g0 + ia, f] = bc[16 * ia:16 * ia + 16]

        if first:
            ya = proj(D, KSPLIT, r)
            wk2_copy.wait()
            y = jnp.concatenate([ya, proj(D + KSPLIT, D - KSPLIT, r)], axis=1)
        else:
            y = proj(D, D, r)
        ymax = jnp.max(jnp.abs(y).reshape(T1 // 8, 8, D), axis=0)
        kmax = ymax if kmax is None else jnp.maximum(kmax, ymax)
        lane = lax.broadcasted_iota(jnp.int32, (T1, 128), 1)
        hi = lane >= 64
        tiles = [y[:, 128 * j:128 * (j + 1)] for j in range(NT5)]
        for j in range(NT5):
            k_s[j, rows2, :] = pltpu.bitcast(jnp.where(lane == ONES_LANE[j], 1.0, tiles[j]).astype(bf16), u32)
        for j in range(NT5 - 1):
            seam = jnp.where(hi, tiles[j], tiles[j + 1])
            k_s[NT5 + j, rows2, :] = pltpu.bitcast(
                jnp.where(lane == ONES_LANE[NT5 + j], 1.0, seam).astype(bf16), u32)
        krs = [y[a * KC + KC - 16:a * KC + KC, :].astype(bf16).astype(f32) for a in APC]
        if first:
            wv_copy.wait()
            wq_copy.wait()
            for tt in range(1, N1):
                x_copy(tt).start()
        kb_gen(krs, 0, D // 2)
        vT = proj(2 * D, D, r).astype(bf16).T.astype(f32)
        lo4 = lax.broadcasted_iota(jnp.int32, (8, T1), 0) < 4
        for p in range(H // 2):
            vT_s[48 * p:48 * p + 16, rows] = vT[40 * p:40 * p + 16]
            mid = vT[40 * p + 16:40 * p + 24]
            vT_s[48 * p + 16:48 * p + 24, rows] = jnp.where(lo4, mid, 1.0)
            vT_s[48 * p + 24:48 * p + 32, rows] = jnp.where(lo4, 1.0, mid)
            vT_s[48 * p + 32:48 * p + 48, rows] = vT[40 * p + 24:40 * p + 40]
        kb_gen(krs, D // 2, D)
        qT = proj(0, D, r * QSCALE).astype(bf16).T
        qT_s[:, rows] = pltpu.bitcast(qT, u32)
        qTf_s[:, rows] = qT.astype(f32)
        return kmax

    def p1(t, kmax):
        x_copy(t).wait()
        return p1_chunk(t, False, kmax)

    wk2_copy.start()
    x_copy(0).wait()
    wk1_copy.wait()
    wv_copy.start()
    wq_copy.start()
    kmax0 = p1_chunk(0, True, None)
    wo_copy.start()
    w1_copy.start()
    w2_copy.start()
    b1_copy.start()
    b2_copy.start()
    kmax = lax.fori_loop(1, N1, p1, kmax0)
    km = jnp.max(kmax, axis=0, keepdims=True) * (1.0 + 2.0 ** -7)
    kmx_s[...] = jnp.broadcast_to(km, (128, D)).T

    tmask = [None]
    zbits = {}

    def zbit(k):
        if k not in zbits:
            zbits[k] = zero_s[k] & 1
        return zbits[k]

    def new_block():
        zbits.clear()
        tmask[0] = (lax.broadcasted_iota(jnp.int32, (8, 128), 1) + zero_s[0]) >= 0

    def unit_m(pr, par, qb):
        rq = pl.ds(_dyn(40 * pr + 16 * par, 8), VR)
        wf = qTf_s[rq, _rows(qb, TQ)]
        kb = kmx_s[rq, :]
        prod = jnp.abs(wf) * jnp.concatenate([kb] * (TQ // 128), axis=1)
        r24 = lax.broadcasted_iota(jnp.int32, (VR, TQ), 0)
        valid = (r24 >= 4) if par else (r24 < DH)
        mneg = MOFF - jnp.sum(jnp.where(valid, prod, 0.0), axis=0, keepdims=True)
        return jnp.broadcast_to(mneg.astype(bf16).astype(f32), (8, TQ))

    def unit_q(pr, par, qb, mneg8):
        h = 2 * pr + par
        off = (h * DH) % 128
        t = (h * DH) // 128
        strad = off > 128 - DH
        tile = t + _sel(strad, NT5, 0)
        olp = _sel(strad, 32, _sel(t == NT5 - 1, 0, 63))
        qcols = _rows(qb, TQ)
        ra = pl.ds(_dyn(64 * t + _sel(strad, 64, 0), 32), 32)
        rb = pl.ds(_dyn(64 * t + 32, 32), 32)
        w = jnp.concatenate([qT_s[ra, qcols], qT_s[rb, qcols]], axis=0)
        r = lax.broadcasted_iota(jnp.int32, (64, TQ), 0)
        msk = ((2 * r - off + 128) & 127) < DH
        if mneg8 is None:
            other = jnp.zeros((64, TQ), u32)
        else:
            mb = pltpu.bitcast(mneg8, u32)
            other = jnp.where(r == olp, jnp.concatenate([mb] * 8, axis=0), jnp.zeros((), u32))
        qm = pltpu.bitcast(jnp.where(msk, w, other), bf16)
        return qm, tile, (par, qb, mneg8, {"rq0": 40 * pr + 16 * par, "hd": h * DH})

    def vpu_sum(info, g, j, d0, nd, init):
        par, qb, _, cache = info
        o4 = 4 * par
        if ("rq", g) not in cache:
            z8 = zbit(16 + g) * 8
            cache[("rq", g)] = pl.multiple_of(cache["rq0"] - z8 if par else cache["rq0"] + z8, 8)
        wf = qTf_s[pl.ds(cache[("rq", g)], VR), pl.ds(qb * TQ + 128 * j, 128)]
        if ("gz", g, j) not in cache:
            z1 = zbit(4 * qb + j)
            cache[("gz", g, j)] = g + z1 if g + 1 < NGRP else g - z1
        kb = kb_all[cache[("gz", g, j)], pl.ds(cache["hd"] + d0, nd)].reshape(nd, 2, 8, 128)
        qb_ = lax.concatenate(
            [lax.broadcast_in_dim(lax.slice(wf, (o4 + d, 0), (o4 + d + 1, 128)), (1, 1, 8, 128), (2, 3))
             for d in range(d0, d0 + nd)], 0)
        prod = kb * qb_
        cuts = [(i * nd) // NCH for i in range(NCH + 1)]
        parts = [jnp.sum(prod[a:b], axis=0) for a, b in zip(cuts[:-1], cuts[1:]) if b > a]
        parts[0] = parts[0] + init
        while len(parts) > 1:
            parts = [parts[k] + parts[k + 1] if k + 1 < len(parts) else parts[k] for k in range(0, len(parts), 2)]
        return parts[0]

    def step_qk(uq, c, extra_pins):
        qm, tile, info = uq
        nm = KC - 16 if c in ASSIST else KC
        ku = k_s[tile, pl.ds(c * KC // 2, nm // 2), :]
        pins = []
        wk = WORK_AT[c]
        i = 0
        while i < len(wk):
            pos, (g, j, k) = wk[i]
            dst = (pl.ds(ASSIST[g] * KC + KC - 16, 16), slice(128 * j, 128 * (j + 1)))
            nq = 1
            i += 1
            while i < len(wk) and wk[i][0] == pos and wk[i][1][:2] == (g, j):
                nq += 1
                i += 1
            if k > 0:
                init = sA[dst].reshape(2, 8, 128)
            else:
                init = info[2][None, :, 128 * j:128 * (j + 1)]
            v = vpu_sum(info, g, j, 5 * k, 5 * nq, init)
            sA[dst] = v.reshape(16, 128)
            pins.append((pos, v[0]))
            pins.append((pos, v[1]))
        pins += extra_pins
        pvpins = [v for pos, v in pins if pos == 9]
        pins = [(pos, v) for pos, v in pins if pos != 9]
        if pins:
            parts = [ku[8 * j:8 * j + 8] for j in range(nm // 16)]
            for pos, v in pins:
                parts[pos] = lax.select(tmask[0], parts[pos], pltpu.bitcast(v, u32))
            ku = jnp.concatenate(parts, axis=0)
        sA[pl.ds(c * KC, nm), :] = jnp.dot(pltpu.bitcast(ku, bf16), qm, preferred_element_type=f32)
        return pvpins

    def store_o(acc, pr, par, qb):
        orow = _dyn(pr * 40, 8)
        qcols = _rows(qb, TQ)
        if par == 0:
            l = acc[DH:DH + 1, :]
            oT_s[pl.ds(orow, VR), qcols] = acc * (1.0 / l)
        else:
            l = acc[0:1, :]
            o = acc * (1.0 / l)
            lo4 = lax.broadcasted_iota(jnp.int32, (8, TQ), 0) < 4
            mid_e = oT_s[pl.ds(orow + 16, 8), qcols]
            oT_s[pl.ds(orow + 16, 8), qcols] = jnp.where(lo4, mid_e, o[0:8])
            oT_s[pl.ds(orow + 24, 16), qcols] = o[8:24]
        return l

    new_block()
    m0 = unit_m(0, 0, 0)
    uq0 = unit_q(0, 0, 0, m0)
    for c in range(LAG):
        step_qk(uq0, c, [])

    def body(p, carry):
        ok, m_cur = carry
        new_block()
        pn = jnp.minimum(p + 1, H // 2 - 1)
        acc = None
        uq = None
        ms = {0: m_cur}
        for n in range(8 * NSTEP):
            ka, ca = divmod(n + LAG, NSTEP)
            if ca == 0 or n == 0:
                uq = unit_q(p if ka < 8 else pn, (ka % 8) // 4, ka % 4, ms[ka])
            extra = []
            if ca == MSTEP and ka < 8:
                k2 = ka + 1
                ms[k2] = unit_m(p if k2 < 8 else pn, (k2 % 8) // 4, k2 % 4)
                extra = [(9, ms[k2][:, 128 * j:128 * (j + 1)]) for j in range(TQ // 128)]
            pvpins = step_qk(uq, ca, extra)
            kb_, cb = divmod(n, NSTEP)
            par, qb = kb_ // 4, kb_ % 4
            vrow = pl.multiple_of(p * 48 + 24 * par, 8)
            pp = jnp.exp2(sA[pl.ds(cb * KC, KC), :]).astype(bf16)
            vt = vT_s[pl.ds(vrow, VR), pl.ds(cb * KC, KC)]
            if pvpins:
                v0 = vt[0:8]
                for v in pvpins:
                    v0 = lax.select(tmask[0], v0, v)
                vt = jnp.concatenate([v0, vt[8:]], axis=0)
            r = jnp.dot(vt, pp, preferred_element_type=f32)
            if cb == 0:
                acc = jnp.full((VR, TQ), zero_s[1].astype(f32), f32) + r
            else:
                acc = acc + r
            if cb == NSTEP - 1:
                l = store_o(acc, p, par, qb)
                aa = jnp.abs(acc)
                big = jnp.maximum(jnp.maximum(aa[0:8], aa[8:16]), aa[16:24])
                good = jnp.logical_and(big <= AMAX, l >= LMIN)
                ok = jnp.minimum(ok, jnp.where(good, 1.0, -1.0))
        return ok, ms[8]

    ok, _ = lax.fori_loop(0, H // 2, body, (jnp.ones((8, TQ), f32), m0))

    @pl.when(jnp.min(ok) < 0.0)
    def _fallback():
        def unit(u, c0):
            pr = u // 8
            for par in range(2):
                @pl.when((u // 4) % 2 == par)
                def _():
                    qb = u % 4
                    qm, tile, _info = unit_q(pr, par, qb, None)

                    def pass1(c, m8):
                        kk = pltpu.bitcast(k_s[tile, _rows(c, KC // 2), :], bf16)
                        s = jnp.dot(kk, qm, preferred_element_type=f32)
                        sA[_rows(c, KC), :] = s
                        return jnp.maximum(m8, jnp.max(s.reshape(KC // 8, 8, TQ), axis=0))
                    m8 = lax.fori_loop(0, NSTEP, pass1, jnp.full((8, TQ), -jnp.inf, f32))
                    m = jnp.max(m8, axis=0, keepdims=True)
                    vrow = pl.multiple_of(pr * 48 + 24 * par, 8)

                    def pass2(c, acc):
                        krows = _rows(c, KC)
                        pp = jnp.exp2(sA[krows, :] - m).astype(bf16)
                        return acc + jnp.dot(vT_s[pl.ds(vrow, VR), krows], pp, preferred_element_type=f32)
                    acc = lax.fori_loop(0, NSTEP, pass2, jnp.zeros((VR, TQ), f32))
                    store_o(acc, pr, par, qb)
            return c0
        lax.fori_loop(0, H * NQ, unit, 0)

    wo_copy.wait()
    w1_copy.wait()
    w2_copy.wait()
    b1_copy.wait()
    b2_copy.wait()

    def out_copy(g):
        slot = g % (2 * NH3)
        return pltpu.make_async_copy(out_s.at[slot], o_hbm.at[_rows(g, T3), :], sem_o.at[slot])

    def p3(trip, c):
        @pl.when(trip >= 2)
        def _():
            for k in range(NH3):
                out_copy((trip - 2) * NH3 + k).wait()

        b1 = b1_ref[...].reshape(1, F).astype(f32)
        b2 = b2_ref[...].reshape(1, D).astype(f32)
        hres = []
        for k in range(NH3):
            rows = _rows(trip * NH3 + k, T3)
            oT = oT_s[:, rows].astype(bf16)
            attn = lax.dot_general(oT, wo_s[...], TN, preferred_element_type=f32)
            hres.append(x_s[rows, :].astype(f32) + attn)
        act = []
        for k in range(NH3):
            hn = _ln(hres[k]).astype(bf16)
            a = jnp.dot(hn, w1_s[...], preferred_element_type=f32) + b1
            act.append(_gelu(a).astype(bf16))
        for k in range(NH3):
            g = trip * NH3 + k
            y = jnp.dot(act[k], w2_s[...], preferred_element_type=f32) + b2
            out_s[g % (2 * NH3)] = (hres[k] + y).astype(bf16)
            out_copy(g).start()
        return c

    lax.fori_loop(0, S // (T3 * NH3), p3, 0)
    for g in range(S // T3 - 2 * NH3, S // T3):
        out_copy(g).wait()


@jax.jit
def pallas_sequential_preLN__softmax_full_mha__dense_activation_gelu__prompt_kernel(
    A_x: jax.Array,
    A_wqkv: jax.Array,
    A_wo: jax.Array,
    B_x: jax.Array,
    B_w1: jax.Array,
    B_b1: jax.Array,
    B_w2: jax.Array,
    B_b2: jax.Array,
):
    anyspec = pl.BlockSpec(memory_space=pl.ANY)
    out = pl.pallas_call(
        _kernel,
        in_specs=[anyspec] * 7,
        out_specs=anyspec,
        out_shape=jax.ShapeDtypeStruct((S, D), bf16),
        scratch_shapes=[
            pltpu.VMEM((S, D), bf16),
            pltpu.VMEM((D, 3 * D), bf16),
            pltpu.VMEM((D, D), bf16),
            pltpu.VMEM((D, F), bf16),
            pltpu.VMEM((F, D), bf16),
            pltpu.VMEM((NTILE, S // 2, 128), u32),
            pltpu.VMEM((D // 2, S), u32),
            pltpu.VMEM((D, S), f32),
            pltpu.VMEM((DV, S), f32),
            pltpu.VMEM((S, TQ), f32),
            pltpu.VMEM((D, S), f32),
            pltpu.VMEM((2 * NH3, T3, D), bf16),
            pltpu.VMEM((F,), bf16),
            pltpu.VMEM((D,), bf16),
            pltpu.VMEM((1, 2944), f32),
            pltpu.VMEM((NGRP, D, 16, 128), f32),
            pltpu.VMEM((D, 128), f32),
            pltpu.SMEM((64,), jnp.int32),
            pltpu.SemaphoreType.DMA((N1,)),
            pltpu.SemaphoreType.DMA((9,)),
            pltpu.SemaphoreType.DMA((2 * NH3,)),
        ],
        compiler_params=pltpu.CompilerParams(vmem_limit_bytes=112 * 1024 * 1024),
    )(A_x.reshape(S, D), A_wqkv, A_wo, B_w1, B_w2, B_b1, B_b2)
    return out.reshape(1, S, D)
```

```python
import functools
import math

import jax
import jax.numpy as jnp
from jax import lax
import jax.experimental.pallas as pl
import jax.experimental.pallas.tpu as pltpu

S = 2048
D = 640
H = 32
DH = 20
F = 1536
NT5 = D // 128
NTILE = 9
VR = 24
DV = H * VR
TQ = 512
NQ = S // TQ
KC = 128
NSTEP = S // KC
EPS = 1e-5
QSCALE = (DH ** -0.5) * math.log2(math.e)
MOFF = 40.0
LMIN = 2.0 ** -80
AMAX = 2.0 ** 120
ONES_LANE = (127, 127, 127, 127, 1, 65, 65, 65, 65)

T1 = 512
N1 = S // T1
KSPLIT = 256
T3 = 256
NH3 = 2
LAG = 4
APC = (1, 2, 3)
ASSIST = tuple(t * (T1 // KC) + a for t in range(N1) for a in APC)
NGRP = len(ASSIST)
SLOTS7 = ((0, 1), (1, 1), (2, 2), (3, 2), (4, 2), (5, 2), (6, 2), (9, 1))
SLOTS8 = ((0, 1), (1, 1), (2, 2), (3, 2), (4, 2), (5, 2), (6, 2), (7, 2), (9, 1))
SLOTS_AT = {4: ((3, 2), (4, 2), (5, 2), (6, 2)), 5: ((5, 2), (6, 2))}
MSTEP = 13
NCH = 2
KBB = 32

TN = (((0,), (0,)), ((), ()))
f32 = jnp.float32
bf16 = jnp.bfloat16
u32 = jnp.uint32


def _plan_vpu_work():
    quanta = [(g, j, k) for g in range(NGRP) for j in range(TQ // 128) for k in range(4)]
    work_at = {}
    i = 0
    for c in range(NSTEP):
        lst = []
        for pos, w in SLOTS_AT.get(c, SLOTS7 if c in ASSIST else SLOTS8):
            take = quanta[i:i + w]
            i += len(take)
            for qn in take:
                assert ASSIST[qn[0]] + LAG - 2 >= c >= ASSIST[qn[0]] + LAG - 14
                lst.append((pos, qn))
        work_at[c] = lst
    assert i == len(quanta)
    return work_at


WORK_AT = _plan_vpu_work()


def _ln(x):
    m = jnp.mean(x, axis=-1, keepdims=True)
    xc = x - m
    v = jnp.mean(xc * xc, axis=-1, keepdims=True)
    return xc * lax.rsqrt(v + EPS)


def _gelu(x):
    c = math.sqrt(2.0 / math.pi)
    return 0.5 * x * (1.0 + jnp.tanh(c * (x + 0.044715 * (x * x * x))))


def _rows(t, size):
    return pl.ds(t * size, size) if isinstance(t, int) else pl.ds(pl.multiple_of(t * size, size), size)


def _dyn(v, m):
    return v if isinstance(v, int) else pl.multiple_of(v, m)


def _sel(c, a, b):
    return (a if c else b) if isinstance(c, bool) else jnp.where(c, a, b)


def _kernel(x_hbm, wqkv_hbm, wo_hbm, w1_hbm, w2_hbm, b1_hbm, b2_hbm, o_hbm,
            x_s, wqkv_s, wo_s, w1_s, w2_s, k_s, qT_s, qTf_s, vT_s, sA, oT_s, out_s, b1_ref, b2_ref, cs_s,
            kb_all, kmx_s, zero_s, sem_x, sem_w, sem_o):

    def x_copy(t):
        rows = _rows(t, T1)
        return pltpu.make_async_copy(x_hbm.at[rows, :], x_s.at[rows, :], sem_x.at[t])

    def wcols_copy(lo, n, sem):
        cols = pl.ds(lo, n)
        return pltpu.make_async_copy(wqkv_hbm.at[:, cols], wqkv_s.at[:, cols], sem_w.at[sem])

    wk1_copy = wcols_copy(D, KSPLIT, 0)
    wk2_copy = wcols_copy(D + KSPLIT, D - KSPLIT, 1)
    wv_copy = wcols_copy(2 * D, D, 2)
    wq_copy = wcols_copy(0, D, 3)
    wo_copy = pltpu.make_async_copy(wo_hbm, wo_s, sem_w.at[4])
    w1_copy = pltpu.make_async_copy(w1_hbm, w1_s, sem_w.at[5])
    w2_copy = pltpu.make_async_copy(w2_hbm, w2_s, sem_w.at[6])
    b1_copy = pltpu.make_async_copy(b1_hbm, b1_ref, sem_w.at[7])
    b2_copy = pltpu.make_async_copy(b2_hbm, b2_ref, sem_w.at[8])

    x_copy(0).start()
    wk1_copy.start()
    for k in range(64):
        zero_s[k] = 0

    def p1_chunk(t, first, kmax):
        rows = _rows(t, T1)
        rows2 = _rows(t, T1 // 2)
        xb = x_s[rows, :]
        xf = xb.astype(f32)
        mu = jnp.mean(xf, axis=-1, keepdims=True)
        xc = xf - mu
        r = lax.rsqrt(jnp.mean(xc * xc, axis=-1, keepdims=True) + EPS)
        if first:
            xb = jnp.concatenate([jnp.ones((16, D), bf16), xb], axis=0)

        def proj(lo, n, rr):
            cols = slice(lo, lo + n)
            y = jnp.dot(xb, wqkv_s[:, cols], preferred_element_type=f32)
            if first:
                c = y[0:1]
                cs_s[:, cols] = c
                y = y[16:]
            else:
                c = cs_s[:, cols]
            return (y - mu * c) * rr

        def kb_gen(krs, f0, f1):
            na = len(krs)
            kr = jnp.concatenate(krs, axis=0)
            for fb in range(f0, f1, KBB):
                bc = [lax.broadcast_in_dim(lax.slice(kr, (0, f), (16 * na, f + 1)), (16 * na, 128), (0, 1))
                      .reshape(na, 1, 16, 128) for f in range(fb, fb + KBB)]
                kb_all[_rows(t, na), fb:fb + KBB] = lax.concatenate(bc, 1)

        if first:
            ya = proj(D, KSPLIT, r)
            wk2_copy.wait()
            y = jnp.concatenate([ya, proj(D + KSPLIT, D - KSPLIT, r)], axis=1)
        else:
            y = proj(D, D, r)
        ymax = jnp.max(jnp.abs(y).reshape(T1 // 8, 8, D), axis=0)
        kmax = ymax if kmax is None else jnp.maximum(kmax, ymax)
        lane = lax.broadcasted_iota(jnp.int32, (T1, 128), 1)
        hi = lane >= 64
        tiles = [y[:, 128 * j:128 * (j + 1)] for j in range(NT5)]
        for j in range(NT5):
            k_s[j, rows2, :] = pltpu.bitcast(jnp.where(lane == ONES_LANE[j], 1.0, tiles[j]).astype(bf16), u32)
        for j in range(NT5 - 1):
            seam = jnp.where(hi, tiles[j], tiles[j + 1])
            k_s[NT5 + j, rows2, :] = pltpu.bitcast(
                jnp.where(lane == ONES_LANE[NT5 + j], 1.0, seam).astype(bf16), u32)
        krs = [y[a * KC + KC - 16:a * KC + KC, :].astype(bf16).astype(f32) for a in APC]
        if first:
            wv_copy.wait()
            wq_copy.wait()
            for tt in range(1, N1):
                x_copy(tt).start()
        kb_gen(krs, 0, D // 2)
        vT = proj(2 * D, D, r).astype(bf16).T.astype(f32)
        lo4 = lax.broadcasted_iota(jnp.int32, (8, T1), 0) < 4
        for p in range(H // 2):
            vT_s[48 * p:48 * p + 16, rows] = vT[40 * p:40 * p + 16]
            mid = vT[40 * p + 16:40 * p + 24]
            vT_s[48 * p + 16:48 * p + 24, rows] = jnp.where(lo4, mid, 1.0)
            vT_s[48 * p + 24:48 * p + 32, rows] = jnp.where(lo4, 1.0, mid)
            vT_s[48 * p + 32:48 * p + 48, rows] = vT[40 * p + 24:40 * p + 40]
        kb_gen(krs, D // 2, D)
        qT = proj(0, D, r * QSCALE).astype(bf16).T
        qT_s[:, rows] = pltpu.bitcast(qT, u32)
        qTf_s[:, rows] = qT.astype(f32)
        return kmax

    def p1(t, kmax):
        x_copy(t).wait()
        return p1_chunk(t, False, kmax)

    wk2_copy.start()
    x_copy(0).wait()
    wk1_copy.wait()
    wv_copy.start()
    wq_copy.start()
    kmax0 = p1_chunk(0, True, None)
    wo_copy.start()
    w1_copy.start()
    w2_copy.start()
    b1_copy.start()
    b2_copy.start()
    kmax = lax.fori_loop(1, N1, p1, kmax0)
    km = jnp.max(kmax, axis=0, keepdims=True) * (1.0 + 2.0 ** -7)
    kmx_s[...] = jnp.broadcast_to(km, (128, D)).T

    tmask = [None]
    zbits = {}

    def zbit(k):
        if k not in zbits:
            zbits[k] = zero_s[k] & 1
        return zbits[k]

    def new_block():
        zbits.clear()
        tmask[0] = (lax.broadcasted_iota(jnp.int32, (8, 128), 1) + zero_s[0]) >= 0

    def unit_m(pr, par, qb):
        rq = pl.ds(_dyn(40 * pr + 16 * par, 8), VR)
        wf = qTf_s[rq, _rows(qb, TQ)]
        kb = kmx_s[rq, :]
        prod = jnp.abs(wf) * jnp.concatenate([kb] * (TQ // 128), axis=1)
        r24 = lax.broadcasted_iota(jnp.int32, (VR, TQ), 0)
        valid = (r24 >= 4) if par else (r24 < DH)
        mneg = MOFF - jnp.sum(jnp.where(valid, prod, 0.0), axis=0, keepdims=True)
        return jnp.broadcast_to(mneg.astype(bf16).astype(f32), (8, TQ))

    def unit_q(pr, par, qb, mneg8):
        h = 2 * pr + par
        off = (h * DH) % 128
        t = (h * DH) // 128
        strad = off > 128 - DH
        tile = t + _sel(strad, NT5, 0)
        olp = _sel(strad, 32, _sel(t == NT5 - 1, 0, 63))
        qcols = _rows(qb, TQ)
        ra = pl.ds(_dyn(64 * t + _sel(strad, 64, 0), 32), 32)
        rb = pl.ds(_dyn(64 * t + 32, 32), 32)
        w = jnp.concatenate([qT_s[ra, qcols], qT_s[rb, qcols]], axis=0)
        r = lax.broadcasted_iota(jnp.int32, (64, TQ), 0)
        msk = ((2 * r - off + 128) & 127) < DH
        if mneg8 is None:
            other = jnp.zeros((64, TQ), u32)
        else:
            mb = pltpu.bitcast(mneg8, u32)
            other = jnp.where(r == olp, jnp.concatenate([mb] * 8, axis=0), jnp.zeros((), u32))
        qm = pltpu.bitcast(jnp.where(msk, w, other), bf16)
        return qm, tile, (par, qb, mneg8, {"rq0": 40 * pr + 16 * par, "hd": h * DH})

    def vpu_sum(info, g, j, d0, nd, init):
        par, qb, _, cache = info
        o4 = 4 * par
        if ("rq", g) not in cache:
            z8 = zbit(16 + g) * 8
            cache[("rq", g)] = pl.multiple_of(cache["rq0"] - z8 if par else cache["rq0"] + z8, 8)
        if ("ops", g, j) not in cache:
            z1 = zbit(4 * qb + j)
            gz = g + z1 if g + 1 < NGRP else g - z1
            cache[("ops", g, j)] = (
                qTf_s[pl.ds(cache[("rq", g)], VR), pl.ds(qb * TQ + 128 * j, 128)],
                kb_all[gz, pl.ds(cache["hd"], DH)].reshape(DH, 2, 8, 128))
        wf, kb = cache[("ops", g, j)]
        kb = kb[d0:d0 + nd]
        qb_ = lax.concatenate(
            [lax.broadcast_in_dim(lax.slice(wf, (o4 + d, 0), (o4 + d + 1, 128)), (1, 1, 8, 128), (2, 3))
             for d in range(d0, d0 + nd)], 0)
        prod = kb * qb_
        cuts = [(i * nd) // NCH for i in range(NCH + 1)]
        parts = [jnp.sum(prod[a:b], axis=0) for a, b in zip(cuts[:-1], cuts[1:]) if b > a]
        parts[0] = parts[0] + init
        while len(parts) > 1:
            parts = [parts[k] + parts[k + 1] if k + 1 < len(parts) else parts[k] for k in range(0, len(parts), 2)]
        return parts[0]

    def step_qk(uq, c, extra_pins):
        qm, tile, info = uq
        nm = KC - 16 if c in ASSIST else KC
        ku = k_s[tile, pl.ds(c * KC // 2, nm // 2), :]
        pins = []
        wk = WORK_AT[c]
        i = 0
        while i < len(wk):
            pos, (g, j, k) = wk[i]
            dst = (pl.ds(ASSIST[g] * KC + KC - 16, 16), slice(128 * j, 128 * (j + 1)))
            nq = 1
            i += 1
            while i < len(wk) and wk[i][0] == pos and wk[i][1][:2] == (g, j):
                nq += 1
                i += 1
            cache = info[3]
            if k == 0:
                init = info[2][None, :, 128 * j:128 * (j + 1)]
            elif ("part", g, j) in cache:
                init = cache.pop(("part", g, j))
            else:
                init = sA[dst].reshape(2, 8, 128)
            v = vpu_sum(info, g, j, 5 * k, 5 * nq, init)
            if k + nq == 4 or (c == LAG - 1 and i == len(wk)):
                sA[dst] = v.reshape(16, 128)
            if k + nq < 4:
                cache[("part", g, j)] = v
            pins.append((pos, v[0]))
            pins.append((pos, v[1]))
        pins += extra_pins
        pvpins = [v for pos, v in pins if pos == 9]
        pins = [(pos, v) for pos, v in pins if pos != 9]
        if pins:
            parts = [ku[8 * j:8 * j + 8] for j in range(nm // 16)]
            for pos, v in pins:
                parts[pos] = lax.select(tmask[0], parts[pos], pltpu.bitcast(v, u32))
            ku = jnp.concatenate(parts, axis=0)
        sA[pl.ds(c * KC, nm), :] = jnp.dot(pltpu.bitcast(ku, bf16), qm, preferred_element_type=f32)
        return pvpins

    def store_o(acc, pr, par, qb):
        orow = _dyn(pr * 40, 8)
        qcols = _rows(qb, TQ)
        if par == 0:
            l = acc[DH:DH + 1, :]
            oT_s[pl.ds(orow, VR), qcols] = acc * (1.0 / l)
        else:
            l = acc[0:1, :]
            o = acc * (1.0 / l)
            lo4 = lax.broadcasted_iota(jnp.int32, (8, TQ), 0) < 4
            mid_e = oT_s[pl.ds(orow + 16, 8), qcols]
            oT_s[pl.ds(orow + 16, 8), qcols] = jnp.where(lo4, mid_e, o[0:8])
            oT_s[pl.ds(orow + 24, 16), qcols] = o[8:24]
        return l

    new_block()
    m0 = unit_m(0, 0, 0)
    uq0 = unit_q(0, 0, 0, m0)
    for c in range(LAG):
        step_qk(uq0, c, [])

    def body(p, carry):
        ok, m_cur = carry
        new_block()
        pn = jnp.minimum(p + 1, H // 2 - 1)
        acc = None
        uq = None
        ms = {0: m_cur}
        for n in range(8 * NSTEP):
            ka, ca = divmod(n + LAG, NSTEP)
            if ca == 0 or n == 0:
                uq = unit_q(p if ka < 8 else pn, (ka % 8) // 4, ka % 4, ms[ka])
            extra = []
            if ca == MSTEP and ka < 8:
                k2 = ka + 1
                ms[k2] = unit_m(p if k2 < 8 else pn, (k2 % 8) // 4, k2 % 4)
                extra = [(9, ms[k2][:, 128 * j:128 * (j + 1)]) for j in range(TQ // 128)]
            pvpins = step_qk(uq, ca, extra)
            kb_, cb = divmod(n, NSTEP)
            par, qb = kb_ // 4, kb_ % 4
            vrow = pl.multiple_of(p * 48 + 24 * par, 8)
            pp = jnp.exp2(sA[pl.ds(cb * KC, KC), :]).astype(bf16)
            vt = vT_s[pl.ds(vrow, VR), pl.ds(cb * KC, KC)]
            if pvpins:
                v0 = vt[0:8]
                for v in pvpins:
                    v0 = lax.select(tmask[0], v0, v)
                vt = jnp.concatenate([v0, vt[8:]], axis=0)
            r = jnp.dot(vt, pp, preferred_element_type=f32)
            if cb == 0:
                acc = jnp.full((VR, TQ), zero_s[1].astype(f32), f32) + r
            else:
                acc = acc + r
            if cb == NSTEP - 1:
                l = store_o(acc, p, par, qb)
                aa = jnp.abs(acc)
                big = jnp.maximum(jnp.maximum(aa[0:8], aa[8:16]), aa[16:24])
                good = jnp.logical_and(big <= AMAX, l >= LMIN)
                ok = jnp.minimum(ok, jnp.where(good, 1.0, -1.0))
        return ok, ms[8]

    ok, _ = lax.fori_loop(0, H // 2, body, (jnp.ones((8, TQ), f32), m0))

    @pl.when(jnp.min(ok) < 0.0)
    def _fallback():
        def unit(u, c0):
            pr = u // 8
            for par in range(2):
                @pl.when((u // 4) % 2 == par)
                def _():
                    qb = u % 4
                    qm, tile, _info = unit_q(pr, par, qb, None)

                    def pass1(c, m8):
                        kk = pltpu.bitcast(k_s[tile, _rows(c, KC // 2), :], bf16)
                        s = jnp.dot(kk, qm, preferred_element_type=f32)
                        sA[_rows(c, KC), :] = s
                        return jnp.maximum(m8, jnp.max(s.reshape(KC // 8, 8, TQ), axis=0))
                    m8 = lax.fori_loop(0, NSTEP, pass1, jnp.full((8, TQ), -jnp.inf, f32))
                    m = jnp.max(m8, axis=0, keepdims=True)
                    vrow = pl.multiple_of(pr * 48 + 24 * par, 8)

                    def pass2(c, acc):
                        krows = _rows(c, KC)
                        pp = jnp.exp2(sA[krows, :] - m).astype(bf16)
                        return acc + jnp.dot(vT_s[pl.ds(vrow, VR), krows], pp, preferred_element_type=f32)
                    acc = lax.fori_loop(0, NSTEP, pass2, jnp.zeros((VR, TQ), f32))
                    store_o(acc, pr, par, qb)
            return c0
        lax.fori_loop(0, H * NQ, unit, 0)

    wo_copy.wait()
    w1_copy.wait()
    w2_copy.wait()
    b1_copy.wait()
    b2_copy.wait()

    def out_copy(g):
        slot = g % (2 * NH3)
        return pltpu.make_async_copy(out_s.at[slot], o_hbm.at[_rows(g, T3), :], sem_o.at[slot])

    def p3(trip, c):
        @pl.when(trip >= 2)
        def _():
            for k in range(NH3):
                out_copy((trip - 2) * NH3 + k).wait()

        b1 = b1_ref[...].reshape(1, F).astype(f32)
        b2 = b2_ref[...].reshape(1, D).astype(f32)
        hres = []
        for k in range(NH3):
            rows = _rows(trip * NH3 + k, T3)
            oT = oT_s[:, rows].astype(bf16)
            attn = lax.dot_general(oT, wo_s[...], TN, preferred_element_type=f32)
            hres.append(x_s[rows, :].astype(f32) + attn)
        act = []
        for k in range(NH3):
            hn = _ln(hres[k]).astype(bf16)
            a = jnp.dot(hn, w1_s[...], preferred_element_type=f32) + b1
            act.append(_gelu(a).astype(bf16))
        for k in range(NH3):
            g = trip * NH3 + k
            y = jnp.dot(act[k], w2_s[...], preferred_element_type=f32) + b2
            out_s[g % (2 * NH3)] = (hres[k] + y).astype(bf16)
            out_copy(g).start()
        return c

    lax.fori_loop(0, S // (T3 * NH3), p3, 0)
    for g in range(S // T3 - 2 * NH3, S // T3):
        out_copy(g).wait()


@jax.jit
def pallas_sequential_preLN__softmax_full_mha__dense_activation_gelu__prompt_kernel(
    A_x: jax.Array,
    A_wqkv: jax.Array,
    A_wo: jax.Array,
    B_x: jax.Array,
    B_w1: jax.Array,
    B_b1: jax.Array,
    B_w2: jax.Array,
    B_b2: jax.Array,
):
    anyspec = pl.BlockSpec(memory_space=pl.ANY)
    out = pl.pallas_call(
        _kernel,
        in_specs=[anyspec] * 7,
        out_specs=anyspec,
        out_shape=jax.ShapeDtypeStruct((S, D), bf16),
        scratch_shapes=[
            pltpu.VMEM((S, D), bf16),
            pltpu.VMEM((D, 3 * D), bf16),
            pltpu.VMEM((D, D), bf16),
            pltpu.VMEM((D, F), bf16),
            pltpu.VMEM((F, D), bf16),
            pltpu.VMEM((NTILE, S // 2, 128), u32),
            pltpu.VMEM((D // 2, S), u32),
            pltpu.VMEM((D, S), f32),
            pltpu.VMEM((DV, S), f32),
            pltpu.VMEM((S, TQ), f32),
            pltpu.VMEM((D, S), f32),
            pltpu.VMEM((2 * NH3, T3, D), bf16),
            pltpu.VMEM((F,), bf16),
            pltpu.VMEM((D,), bf16),
            pltpu.VMEM((1, 2944), f32),
            pltpu.VMEM((NGRP, D, 16, 128), f32),
            pltpu.VMEM((D, 128), f32),
            pltpu.SMEM((64,), jnp.int32),
            pltpu.SemaphoreType.DMA((N1,)),
            pltpu.SemaphoreType.DMA((9,)),
            pltpu.SemaphoreType.DMA((2 * NH3,)),
        ],
        compiler_params=pltpu.CompilerParams(vmem_limit_bytes=112 * 1024 * 1024),
    )(A_x.reshape(S, D), A_wqkv, A_wo, B_w1, B_w2, B_b1, B_b2)
    return out.reshape(1, S, D)
```

```python
import functools
import math

import jax
import jax.numpy as jnp
from jax import lax
import jax.experimental.pallas as pl
import jax.experimental.pallas.tpu as pltpu

S = 2048
D = 640
H = 32
DH = 20
F = 1536
NT5 = D // 128
NTILE = 9
VR = 24
DV = H * VR
TQ = 512
NQ = S // TQ
KC = 128
NSTEP = S // KC
EPS = 1e-5
QSCALE = (DH ** -0.5) * math.log2(math.e)
MOFF = 40.0
LMIN = 2.0 ** -80
AMAX = 2.0 ** 120
ONES_LANE = (127, 127, 127, 127, 1, 65, 65, 65, 65)

T1 = 512
N1 = S // T1
KSPLIT = 256
KEARLY = 128
T3 = 256
NH3 = 2
LAG = 4
APC = (1, 2, 3)
ASSIST = tuple(t * (T1 // KC) + a for t in range(N1) for a in APC)
NGRP = len(ASSIST)
SLOTS7 = ((0, 1), (1, 1), (2, 2), (3, 2), (4, 2), (5, 2), (6, 2), (9, 1))
SLOTS8 = ((0, 1), (1, 1), (2, 2), (3, 2), (4, 2), (5, 2), (6, 2), (7, 2), (9, 1))
SLOTS_AT = {4: ((2, 2), (3, 2), (4, 2), (5, 2), (6, 2)), 5: ((5, 2), (6, 2))}
MSTEP = 13
NCH = 3
KBB = 32

TN = (((0,), (0,)), ((), ()))
f32 = jnp.float32
bf16 = jnp.bfloat16
u32 = jnp.uint32


def _plan_vpu_work():
    quanta = [(g, j, k) for g in range(NGRP) for j in range(TQ // 128) for k in range(4)]
    work_at = {}
    i = 0
    for c in range(NSTEP):
        lst = []
        for pos, w in SLOTS_AT.get(c, SLOTS7 if c in ASSIST else SLOTS8):
            take = quanta[i:i + w]
            i += len(take)
            for qn in take:
                assert ASSIST[qn[0]] + LAG - 2 >= c >= ASSIST[qn[0]] + LAG - 14
                lst.append((pos, qn))
        work_at[c] = lst
    assert i == len(quanta)
    return work_at


WORK_AT = _plan_vpu_work()


def _ln(x):
    m = jnp.mean(x, axis=-1, keepdims=True)
    xc = x - m
    v = jnp.mean(xc * xc, axis=-1, keepdims=True)
    return xc * lax.rsqrt(v + EPS)


def _gelu(x):
    c = math.sqrt(2.0 / math.pi)
    return 0.5 * x * (1.0 + jnp.tanh(c * (x + 0.044715 * (x * x * x))))


def _rows(t, size):
    return pl.ds(t * size, size) if isinstance(t, int) else pl.ds(pl.multiple_of(t * size, size), size)


def _dyn(v, m):
    return v if isinstance(v, int) else pl.multiple_of(v, m)


def _sel(c, a, b):
    return (a if c else b) if isinstance(c, bool) else jnp.where(c, a, b)


def _kernel(x_hbm, wqkv_hbm, wo_hbm, w1_hbm, w2_hbm, b1_hbm, b2_hbm, o_hbm,
            x_s, wqkv_s, wo_s, w1_s, w2_s, k_s, qT_s, qTf_s, vT_s, sA, oT_s, out_s, b1_ref, b2_ref, cs_s,
            kb_all, kmx_s, zero_s, sem_x, sem_w, sem_o):

    def x_copy(t):
        rows = _rows(t, T1)
        return pltpu.make_async_copy(x_hbm.at[rows, :], x_s.at[rows, :], sem_x.at[t])

    def wcols_copy(lo, n, sem):
        cols = pl.ds(lo, n)
        return pltpu.make_async_copy(wqkv_hbm.at[:, cols], wqkv_s.at[:, cols], sem_w.at[sem])

    wk1_copy = wcols_copy(D, KSPLIT, 0)
    wk2_copy = wcols_copy(D + KSPLIT, D - KSPLIT, 1)
    wv_copy = wcols_copy(2 * D, D, 2)
    wq_copy = wcols_copy(0, D, 3)
    wo_copy = pltpu.make_async_copy(wo_hbm, wo_s, sem_w.at[4])
    w1_copy = pltpu.make_async_copy(w1_hbm, w1_s, sem_w.at[5])
    w2_copy = pltpu.make_async_copy(w2_hbm, w2_s, sem_w.at[6])
    b1_copy = pltpu.make_async_copy(b1_hbm, b1_ref, sem_w.at[7])
    b2_copy = pltpu.make_async_copy(b2_hbm, b2_ref, sem_w.at[8])

    x_copy(0).start()
    wk1_copy.start()
    for k in range(64):
        zero_s[k] = 0

    def p1_chunk(t, first, kmax):
        rows = _rows(t, T1)
        rows2 = _rows(t, T1 // 2)
        xb = x_s[rows, :]
        xf = xb.astype(f32)
        mu = jnp.mean(xf, axis=-1, keepdims=True)
        xc = xf - mu
        r = lax.rsqrt(jnp.mean(xc * xc, axis=-1, keepdims=True) + EPS)
        if first:
            xb = jnp.concatenate([jnp.ones((16, D), bf16), xb], axis=0)

        def proj(lo, n, rr):
            cols = slice(lo, lo + n)
            y = jnp.dot(xb, wqkv_s[:, cols], preferred_element_type=f32)
            if first:
                c = y[0:1]
                cs_s[:, cols] = c
                y = y[16:]
            else:
                c = cs_s[:, cols]
            return (y - mu * c) * rr

        def kb_gen(krs, f0, f1):
            na = len(krs)
            kr = jnp.concatenate(krs, axis=0)
            for fb in range(f0, f1, KBB):
                bc = [lax.broadcast_in_dim(lax.slice(kr, (0, f), (16 * na, f + 1)), (16 * na, 128), (0, 1))
                      .reshape(na, 1, 16, 128) for f in range(fb, fb + KBB)]
                kb_all[_rows(t, na), fb:fb + KBB] = lax.concatenate(bc, 1)

        def vpu_keys(y):
            return [y[a * KC + KC - 16:a * KC + KC, :].astype(bf16).astype(f32) for a in APC]

        if first:
            ya = proj(D, KSPLIT, r)
            wk2_copy.wait()
            kb_gen(vpu_keys(ya), 0, KEARLY)
            y = jnp.concatenate([ya, proj(D + KSPLIT, D - KSPLIT, r)], axis=1)
        else:
            y = proj(D, D, r)
        ymax = jnp.max(jnp.abs(y).reshape(T1 // 8, 8, D), axis=0)
        kmax = ymax if kmax is None else jnp.maximum(kmax, ymax)
        lane = lax.broadcasted_iota(jnp.int32, (T1, 128), 1)
        hi = lane >= 64
        tiles = [y[:, 128 * j:128 * (j + 1)] for j in range(NT5)]
        for j in range(NT5):
            k_s[j, rows2, :] = pltpu.bitcast(jnp.where(lane == ONES_LANE[j], 1.0, tiles[j]).astype(bf16), u32)
        for j in range(NT5 - 1):
            seam = jnp.where(hi, tiles[j], tiles[j + 1])
            k_s[NT5 + j, rows2, :] = pltpu.bitcast(
                jnp.where(lane == ONES_LANE[NT5 + j], 1.0, seam).astype(bf16), u32)
        krs = vpu_keys(y)
        if first:
            wv_copy.wait()
            wq_copy.wait()
            for tt in range(1, N1):
                x_copy(tt).start()
        kb_gen(krs, KEARLY if first else 0, D // 2)
        vT = proj(2 * D, D, r).astype(bf16).T.astype(f32)
        lo4 = lax.broadcasted_iota(jnp.int32, (8, T1), 0) < 4
        for p in range(H // 2):
            vT_s[48 * p:48 * p + 16, rows] = vT[40 * p:40 * p + 16]
            mid = vT[40 * p + 16:40 * p + 24]
            vT_s[48 * p + 16:48 * p + 24, rows] = jnp.where(lo4, mid, 1.0)
            vT_s[48 * p + 24:48 * p + 32, rows] = jnp.where(lo4, 1.0, mid)
            vT_s[48 * p + 32:48 * p + 48, rows] = vT[40 * p + 24:40 * p + 40]
        kb_gen(krs, D // 2, D)
        qT = proj(0, D, r * QSCALE).astype(bf16).T
        qT_s[:, rows] = pltpu.bitcast(qT, u32)
        qTf_s[:, rows] = qT.astype(f32)
        return kmax

    def p1(t, kmax):
        x_copy(t).wait()
        return p1_chunk(t, False, kmax)

    wk2_copy.start()
    x_copy(0).wait()
    wk1_copy.wait()
    wv_copy.start()
    wq_copy.start()
    kmax0 = p1_chunk(0, True, None)
    wo_copy.start()
    w1_copy.start()
    w2_copy.start()
    b1_copy.start()
    b2_copy.start()
    kmax = lax.fori_loop(1, N1, p1, kmax0)
    km = jnp.max(kmax, axis=0, keepdims=True) * (1.0 + 2.0 ** -7)
    kmx_s[...] = jnp.broadcast_to(km, (128, D)).T

    tmask = [None]
    zbits = {}

    def zbit(k):
        if k not in zbits:
            zbits[k] = zero_s[k] & 1
        return zbits[k]

    def new_block():
        zbits.clear()
        tmask[0] = (lax.broadcasted_iota(jnp.int32, (8, 128), 1) + zero_s[0]) >= 0

    def unit_m(pr, par, qb):
        rq = pl.ds(_dyn(40 * pr + 16 * par, 8), VR)
        wf = qTf_s[rq, _rows(qb, TQ)]
        kb = kmx_s[rq, :]
        prod = jnp.abs(wf) * jnp.concatenate([kb] * (TQ // 128), axis=1)
        r24 = lax.broadcasted_iota(jnp.int32, (VR, TQ), 0)
        valid = (r24 >= 4) if par else (r24 < DH)
        mneg = MOFF - jnp.sum(jnp.where(valid, prod, 0.0), axis=0, keepdims=True)
        return jnp.broadcast_to(mneg.astype(bf16).astype(f32), (8, TQ))

    def unit_q(pr, par, qb, mneg8):
        h = 2 * pr + par
        off = (h * DH) % 128
        t = (h * DH) // 128
        strad = off > 128 - DH
        tile = t + _sel(strad, NT5, 0)
        olp = _sel(strad, 32, _sel(t == NT5 - 1, 0, 63))
        qcols = _rows(qb, TQ)
        ra = pl.ds(_dyn(64 * t + _sel(strad, 64, 0), 32), 32)
        rb = pl.ds(_dyn(64 * t + 32, 32), 32)
        w = jnp.concatenate([qT_s[ra, qcols], qT_s[rb, qcols]], axis=0)
        r = lax.broadcasted_iota(jnp.int32, (64, TQ), 0)
        msk = ((2 * r - off + 128) & 127) < DH
        if mneg8 is None:
            other = jnp.zeros((64, TQ), u32)
        else:
            mb = pltpu.bitcast(mneg8, u32)
            other = jnp.where(r == olp, jnp.concatenate([mb] * 8, axis=0), jnp.zeros((), u32))
        qm = pltpu.bitcast(jnp.where(msk, w, other), bf16)
        return qm, tile, (par, qb, mneg8, {"rq0": 40 * pr + 16 * par, "hd": h * DH})

    def vpu_sum(info, g, j, d0, nd, init):
        par, qb, _, cache = info
        o4 = 4 * par
        if ("rq", g) not in cache:
            z8 = zbit(16 + g) * 8
            cache[("rq", g)] = pl.multiple_of(cache["rq0"] - z8 if par else cache["rq0"] + z8, 8)
        if ("ops", g, j) not in cache:
            z1 = zbit(4 * qb + j)
            gz = g + z1 if g + 1 < NGRP else g - z1
            cache[("ops", g, j)] = (
                qTf_s[pl.ds(cache[("rq", g)], VR), pl.ds(qb * TQ + 128 * j, 128)],
                kb_all[gz, pl.ds(cache["hd"], DH)].reshape(DH, 2, 8, 128))
        wf, kb = cache[("ops", g, j)]
        kb = kb[d0:d0 + nd]
        qb_ = lax.concatenate(
            [lax.broadcast_in_dim(lax.slice(wf, (o4 + d, 0), (o4 + d + 1, 128)), (1, 1, 8, 128), (2, 3))
             for d in range(d0, d0 + nd)], 0)
        prod = kb * qb_
        cuts = [(i * nd) // NCH for i in range(NCH + 1)]
        parts = [jnp.sum(prod[a:b], axis=0) for a, b in zip(cuts[:-1], cuts[1:]) if b > a]
        parts[0] = parts[0] + init
        while len(parts) > 1:
            parts = [parts[k] + parts[k + 1] if k + 1 < len(parts) else parts[k] for k in range(0, len(parts), 2)]
        return parts[0]

    def step_qk(uq, c, extra_pins):
        qm, tile, info = uq
        nm = KC - 16 if c in ASSIST else KC
        ku = k_s[tile, pl.ds(c * KC // 2, nm // 2), :]
        pins = []
        wk = WORK_AT[c]
        i = 0
        while i < len(wk):
            pos, (g, j, k) = wk[i]
            dst = (pl.ds(ASSIST[g] * KC + KC - 16, 16), slice(128 * j, 128 * (j + 1)))
            nq = 1
            i += 1
            while i < len(wk) and wk[i][0] == pos and wk[i][1][:2] == (g, j):
                nq += 1
                i += 1
            cache = info[3]
            if k == 0:
                init = info[2][None, :, 128 * j:128 * (j + 1)]
            elif ("part", g, j) in cache:
                init = cache.pop(("part", g, j))
            else:
                init = sA[dst].reshape(2, 8, 128)
            v = vpu_sum(info, g, j, 5 * k, 5 * nq, init)
            if k + nq == 4 or (c == LAG - 1 and i == len(wk)):
                sA[dst] = v.reshape(16, 128)
            if k + nq < 4:
                cache[("part", g, j)] = v
            pins.append((pos, v[0]))
            pins.append((pos, v[1]))
        pins += extra_pins
        pvpins = [v for pos, v in pins if pos == 9]
        pins = [(pos, v) for pos, v in pins if pos != 9]
        if pins:
            parts = [ku[8 * j:8 * j + 8] for j in range(nm // 16)]
            for pos, v in pins:
                parts[pos] = lax.select(tmask[0], parts[pos], pltpu.bitcast(v, u32))
            ku = jnp.concatenate(parts, axis=0)
        sA[pl.ds(c * KC, nm), :] = jnp.dot(pltpu.bitcast(ku, bf16), qm, preferred_element_type=f32)
        return pvpins

    def store_o(acc, pr, par, qb):
        orow = _dyn(pr * 40, 8)
        qcols = _rows(qb, TQ)
        if par == 0:
            l = acc[DH:DH + 1, :]
            oT_s[pl.ds(orow, VR), qcols] = acc * (1.0 / l)
        else:
            l = acc[0:1, :]
            o = acc * (1.0 / l)
            lo4 = lax.broadcasted_iota(jnp.int32, (8, TQ), 0) < 4
            mid_e = oT_s[pl.ds(orow + 16, 8), qcols]
            oT_s[pl.ds(orow + 16, 8), qcols] = jnp.where(lo4, mid_e, o[0:8])
            oT_s[pl.ds(orow + 24, 16), qcols] = o[8:24]
        return l

    new_block()
    m0 = unit_m(0, 0, 0)
    uq0 = unit_q(0, 0, 0, m0)
    for c in range(LAG):
        step_qk(uq0, c, [])

    def body(p, carry):
        ok, m_cur = carry
        new_block()
        pn = jnp.minimum(p + 1, H // 2 - 1)
        acc = None
        uq = None
        ms = {0: m_cur}
        for n in range(8 * NSTEP):
            ka, ca = divmod(n + LAG, NSTEP)
            if ca == 0 or n == 0:
                uq = unit_q(p if ka < 8 else pn, (ka % 8) // 4, ka % 4, ms[ka])
            extra = []
            if ca == MSTEP and ka < 8:
                k2 = ka + 1
                ms[k2] = unit_m(p if k2 < 8 else pn, (k2 % 8) // 4, k2 % 4)
                extra = [(9, ms[k2][:, 128 * j:128 * (j + 1)]) for j in range(TQ // 128)]
            pvpins = step_qk(uq, ca, extra)
            kb_, cb = divmod(n, NSTEP)
            par, qb = kb_ // 4, kb_ % 4
            vrow = pl.multiple_of(p * 48 + 24 * par, 8)
            pp = jnp.exp2(sA[pl.ds(cb * KC, KC), :]).astype(bf16)
            vt = vT_s[pl.ds(vrow, VR), pl.ds(cb * KC, KC)]
            if pvpins:
                v0 = vt[0:8]
                for v in pvpins:
                    v0 = lax.select(tmask[0], v0, v)
                vt = jnp.concatenate([v0, vt[8:]], axis=0)
            r = jnp.dot(vt, pp, preferred_element_type=f32)
            if cb == 0:
                acc = jnp.full((VR, TQ), zero_s[1].astype(f32), f32) + r
            else:
                acc = acc + r
            if cb == NSTEP - 1:
                l = store_o(acc, p, par, qb)
                aa = jnp.abs(acc)
                big = jnp.maximum(jnp.maximum(aa[0:8], aa[8:16]), aa[16:24])
                good = jnp.logical_and(big <= AMAX, l >= LMIN)
                ok = jnp.minimum(ok, jnp.where(good, 1.0, -1.0))
        return ok, ms[8]

    ok, _ = lax.fori_loop(0, H // 2, body, (jnp.ones((8, TQ), f32), m0))

    @pl.when(jnp.min(ok) < 0.0)
    def _fallback():
        def unit(u, c0):
            pr = u // 8
            for par in range(2):
                @pl.when((u // 4) % 2 == par)
                def _():
                    qb = u % 4
                    qm, tile, _info = unit_q(pr, par, qb, None)

                    def pass1(c, m8):
                        kk = pltpu.bitcast(k_s[tile, _rows(c, KC // 2), :], bf16)
                        s = jnp.dot(kk, qm, preferred_element_type=f32)
                        sA[_rows(c, KC), :] = s
                        return jnp.maximum(m8, jnp.max(s.reshape(KC // 8, 8, TQ), axis=0))
                    m8 = lax.fori_loop(0, NSTEP, pass1, jnp.full((8, TQ), -jnp.inf, f32))
                    m = jnp.max(m8, axis=0, keepdims=True)
                    vrow = pl.multiple_of(pr * 48 + 24 * par, 8)

                    def pass2(c, acc):
                        krows = _rows(c, KC)
                        pp = jnp.exp2(sA[krows, :] - m).astype(bf16)
                        return acc + jnp.dot(vT_s[pl.ds(vrow, VR), krows], pp, preferred_element_type=f32)
                    acc = lax.fori_loop(0, NSTEP, pass2, jnp.zeros((VR, TQ), f32))
                    store_o(acc, pr, par, qb)
            return c0
        lax.fori_loop(0, H * NQ, unit, 0)

    wo_copy.wait()
    w1_copy.wait()
    w2_copy.wait()
    b1_copy.wait()
    b2_copy.wait()

    def out_copy(g):
        slot = g % (2 * NH3)
        return pltpu.make_async_copy(out_s.at[slot], o_hbm.at[_rows(g, T3), :], sem_o.at[slot])

    def p3(trip, c):
        @pl.when(trip >= 2)
        def _():
            for k in range(NH3):
                out_copy((trip - 2) * NH3 + k).wait()

        b1 = b1_ref[...].reshape(1, F).astype(f32)
        b2 = b2_ref[...].reshape(1, D).astype(f32)
        hres = []
        for k in range(NH3):
            rows = _rows(trip * NH3 + k, T3)
            oT = oT_s[:, rows].astype(bf16)
            attn = lax.dot_general(oT, wo_s[...], TN, preferred_element_type=f32)
            hres.append(x_s[rows, :].astype(f32) + attn)
        act = []
        for k in range(NH3):
            hn = _ln(hres[k]).astype(bf16)
            a = jnp.dot(hn, w1_s[...], preferred_element_type=f32) + b1
            act.append(_gelu(a).astype(bf16))
        for k in range(NH3):
            g = trip * NH3 + k
            y = jnp.dot(act[k], w2_s[...], preferred_element_type=f32) + b2
            out_s[g % (2 * NH3)] = (hres[k] + y).astype(bf16)
            out_copy(g).start()
        return c

    lax.fori_loop(0, S // (T3 * NH3), p3, 0)
    for g in range(S // T3 - 2 * NH3, S // T3):
        out_copy(g).wait()


@jax.jit
def pallas_sequential_preLN__softmax_full_mha__dense_activation_gelu__prompt_kernel(
    A_x: jax.Array,
    A_wqkv: jax.Array,
    A_wo: jax.Array,
    B_x: jax.Array,
    B_w1: jax.Array,
    B_b1: jax.Array,
    B_w2: jax.Array,
    B_b2: jax.Array,
):
    anyspec = pl.BlockSpec(memory_space=pl.ANY)
    out = pl.pallas_call(
        _kernel,
        in_specs=[anyspec] * 7,
        out_specs=anyspec,
        out_shape=jax.ShapeDtypeStruct((S, D), bf16),
        scratch_shapes=[
            pltpu.VMEM((S, D), bf16),
            pltpu.VMEM((D, 3 * D), bf16),
            pltpu.VMEM((D, D), bf16),
            pltpu.VMEM((D, F), bf16),
            pltpu.VMEM((F, D), bf16),
            pltpu.VMEM((NTILE, S // 2, 128), u32),
            pltpu.VMEM((D // 2, S), u32),
            pltpu.VMEM((D, S), f32),
            pltpu.VMEM((DV, S), f32),
            pltpu.VMEM((S, TQ), f32),
            pltpu.VMEM((D, S), f32),
            pltpu.VMEM((2 * NH3, T3, D), bf16),
            pltpu.VMEM((F,), bf16),
            pltpu.VMEM((D,), bf16),
            pltpu.VMEM((1, 2944), f32),
            pltpu.VMEM((NGRP, D, 16, 128), f32),
            pltpu.VMEM((D, 128), f32),
            pltpu.SMEM((64,), jnp.int32),
            pltpu.SemaphoreType.DMA((N1,)),
            pltpu.SemaphoreType.DMA((9,)),
            pltpu.SemaphoreType.DMA((2 * NH3,)),
        ],
        compiler_params=pltpu.CompilerParams(vmem_limit_bytes=112 * 1024 * 1024),
    )(A_x.reshape(S, D), A_wqkv, A_wo, B_w1, B_w2, B_b1, B_b2)
    return out.reshape(1, S, D)
```

```python
import math

import jax
import jax.numpy as jnp
from jax import lax
import jax.experimental.pallas as pl
import jax.experimental.pallas.tpu as pltpu

S = 2048
D = 640
H = 32
DH = 20
F = 1536
NT5 = D // 128
NTILE = 9
VR = 24
DV = H * VR
TQ = 512
NQ = S // TQ
KC = 128
NSTEP = S // KC
EPS = 1e-5
QSCALE = (DH ** -0.5) * math.log2(math.e)
MOFF = 40.0
LMIN = 2.0 ** -80
AMAX = 2.0 ** 120
ONES_LANE = (127, 127, 127, 127, 1, 65, 65, 65, 65)

T1 = 512
N1 = S // T1
KSPLIT = 256
KEARLY = 128
T3 = 256
NH3 = 2
LAG = 4
APC = (1, 2, 3)
ASSIST = tuple(t * (T1 // KC) + a for t in range(N1) for a in APC)
NGRP = len(ASSIST)
SLOTS7 = ((0, 1), (1, 1), (2, 2), (3, 2), (4, 2), (5, 2), (6, 2), (9, 1))
SLOTS8 = ((0, 1), (1, 1), (2, 2), (3, 2), (4, 2), (5, 2), (6, 2), (7, 2), (9, 1))
SLOTS_AT = {4: ((2, 2), (3, 2), (4, 2), (5, 2), (6, 2)), 5: ((5, 2), (6, 2))}
MSTEP = 13
NCH = 3
KBB = 32

TN = (((0,), (0,)), ((), ()))
f32 = jnp.float32
bf16 = jnp.bfloat16
u32 = jnp.uint32


def _plan_vpu_work():
    quanta = [(g, j, k) for g in range(NGRP) for j in range(TQ // 128) for k in range(4)]
    work_at = {}
    i = 0
    for c in range(NSTEP):
        lst = []
        for pos, w in SLOTS_AT.get(c, SLOTS7 if c in ASSIST else SLOTS8):
            take = quanta[i:i + w]
            i += len(take)
            for qn in take:
                assert ASSIST[qn[0]] + LAG - 2 >= c >= ASSIST[qn[0]] + LAG - 14
                lst.append((pos, qn))
        work_at[c] = lst
    assert i == len(quanta)
    return work_at


WORK_AT = _plan_vpu_work()


def _ln(x):
    m = jnp.mean(x, axis=-1, keepdims=True)
    xc = x - m
    v = jnp.mean(xc * xc, axis=-1, keepdims=True)
    return xc * lax.rsqrt(v + EPS)


def _gelu(x):
    c = math.sqrt(2.0 / math.pi)
    return 0.5 * x * (1.0 + jnp.tanh(c * (x + 0.044715 * (x * x * x))))


def _rows(t, size):
    return pl.ds(t * size, size) if isinstance(t, int) else pl.ds(pl.multiple_of(t * size, size), size)


def _dyn(v, m):
    return v if isinstance(v, int) else pl.multiple_of(v, m)


def _sel(c, a, b):
    return (a if c else b) if isinstance(c, bool) else jnp.where(c, a, b)


def _kernel(x_hbm, wqkv_hbm, wo_hbm, w1_hbm, w2_hbm, b1_hbm, b2_hbm, o_hbm,
            x_s, wqkv_s, wo_s, w1_s, w2_s, k_s, qT_s, qTf_s, vT_s, sA, oT_s, out_s, b1_ref, b2_ref, cs_s,
            kb_all, kmx_s, zero_s, sem_x, sem_w, sem_o):

    def x_copy(t):
        rows = _rows(t, T1)
        return pltpu.make_async_copy(x_hbm.at[rows, :], x_s.at[rows, :], sem_x.at[t])

    def wcols_copy(lo, n, sem):
        cols = pl.ds(lo, n)
        return pltpu.make_async_copy(wqkv_hbm.at[:, cols], wqkv_s.at[:, cols], sem_w.at[sem])

    wk1_copy = wcols_copy(D, KSPLIT, 0)
    wk2_copy = wcols_copy(D + KSPLIT, D - KSPLIT, 1)
    wv_copy = wcols_copy(2 * D, D, 2)
    wq_copy = wcols_copy(0, D, 3)
    wo_copy = pltpu.make_async_copy(wo_hbm, wo_s, sem_w.at[4])
    w1_copy = pltpu.make_async_copy(w1_hbm, w1_s, sem_w.at[5])
    w2_copy = pltpu.make_async_copy(w2_hbm, w2_s, sem_w.at[6])
    b1_copy = pltpu.make_async_copy(b1_hbm, b1_ref, sem_w.at[7])
    b2_copy = pltpu.make_async_copy(b2_hbm, b2_ref, sem_w.at[8])

    x_copy(0).start()
    wk1_copy.start()
    for k in range(64):
        zero_s[k] = 0

    def p1_chunk(t, first, kmax):
        rows = _rows(t, T1)
        rows2 = _rows(t, T1 // 2)
        xb = x_s[rows, :]
        xf = xb.astype(f32)
        mu = jnp.mean(xf, axis=-1, keepdims=True)
        xc = xf - mu
        r = lax.rsqrt(jnp.mean(xc * xc, axis=-1, keepdims=True) + EPS)
        if first:
            xb = jnp.concatenate([jnp.ones((16, D), bf16), xb], axis=0)

        def proj(lo, n, rr):
            cols = slice(lo, lo + n)
            y = jnp.dot(xb, wqkv_s[:, cols], preferred_element_type=f32)
            if first:
                c = y[0:1]
                cs_s[:, cols] = c
                y = y[16:]
            else:
                c = cs_s[:, cols]
            return (y - mu * c) * rr

        def kb_gen(krs, f0, f1):
            na = len(krs)
            kr = jnp.concatenate(krs, axis=0)
            for fb in range(f0, f1, KBB):
                bc = [lax.broadcast_in_dim(lax.slice(kr, (0, f), (16 * na, f + 1)), (16 * na, 128), (0, 1))
                      .reshape(na, 1, 16, 128) for f in range(fb, fb + KBB)]
                kb_all[_rows(t, na), fb:fb + KBB] = lax.concatenate(bc, 1)

        def vpu_keys(y):
            return [y[a * KC + KC - 16:a * KC + KC, :].astype(bf16).astype(f32) for a in APC]

        if first:
            ya = proj(D, KSPLIT, r)
            wk2_copy.wait()
            kb_gen(vpu_keys(ya), 0, KEARLY)
            y = jnp.concatenate([ya, proj(D + KSPLIT, D - KSPLIT, r)], axis=1)
        else:
            y = proj(D, D, r)
        ymax = jnp.max(jnp.abs(y).reshape(T1 // 8, 8, D), axis=0)
        kmax = ymax if kmax is None else jnp.maximum(kmax, ymax)
        lane = lax.broadcasted_iota(jnp.int32, (T1, 128), 1)
        hi = lane >= 64
        tiles = [y[:, 128 * j:128 * (j + 1)] for j in range(NT5)]
        for j in range(NT5):
            k_s[j, rows2, :] = pltpu.bitcast(jnp.where(lane == ONES_LANE[j], 1.0, tiles[j]).astype(bf16), u32)
        for j in range(NT5 - 1):
            seam = jnp.where(hi, tiles[j], tiles[j + 1])
            k_s[NT5 + j, rows2, :] = pltpu.bitcast(
                jnp.where(lane == ONES_LANE[NT5 + j], 1.0, seam).astype(bf16), u32)
        krs = vpu_keys(y)
        if first:
            wv_copy.wait()
            wq_copy.wait()
            for tt in range(1, N1):
                x_copy(tt).start()
        kb_gen(krs, KEARLY if first else 0, D // 2)
        vT = proj(2 * D, D, r).astype(bf16).T.astype(f32)
        lo4 = lax.broadcasted_iota(jnp.int32, (8, T1), 0) < 4
        for p in range(H // 2):
            vT_s[48 * p:48 * p + 16, rows] = vT[40 * p:40 * p + 16]
            mid = vT[40 * p + 16:40 * p + 24]
            vT_s[48 * p + 16:48 * p + 24, rows] = jnp.where(lo4, mid, 1.0)
            vT_s[48 * p + 24:48 * p + 32, rows] = jnp.where(lo4, 1.0, mid)
            vT_s[48 * p + 32:48 * p + 48, rows] = vT[40 * p + 24:40 * p + 40]
        kb_gen(krs, D // 2, D)
        qT = proj(0, D, r * QSCALE).astype(bf16).T
        qT_s[:, rows] = pltpu.bitcast(qT, u32)
        qTf_s[:, rows] = qT.astype(f32)
        return kmax

    def p1(t, kmax):
        x_copy(t).wait()
        return p1_chunk(t, False, kmax)

    wk2_copy.start()
    x_copy(0).wait()
    wk1_copy.wait()
    wv_copy.start()
    wq_copy.start()
    kmax0 = p1_chunk(0, True, None)
    wo_copy.start()
    w1_copy.start()
    w2_copy.start()
    b1_copy.start()
    b2_copy.start()
    kmax = lax.fori_loop(1, N1, p1, kmax0)
    km = jnp.max(kmax, axis=0, keepdims=True) * (1.0 + 2.0 ** -7)
    kmx_s[...] = jnp.broadcast_to(km, (128, D)).T

    tmask = [None]
    zbits = {}

    def zbit(k):
        if k not in zbits:
            zbits[k] = zero_s[k] & 1
        return zbits[k]

    def new_block():
        zbits.clear()
        tmask[0] = (lax.broadcasted_iota(jnp.int32, (8, 128), 1) + zero_s[0]) >= 0

    def unit_m(pr, par, qb):
        rq = pl.ds(_dyn(40 * pr + 16 * par, 8), VR)
        wf = qTf_s[rq, _rows(qb, TQ)]
        kb = kmx_s[rq, :]
        prod = jnp.abs(wf) * jnp.concatenate([kb] * (TQ // 128), axis=1)
        r24 = lax.broadcasted_iota(jnp.int32, (VR, TQ), 0)
        valid = (r24 >= 4) if par else (r24 < DH)
        mneg = MOFF - jnp.sum(jnp.where(valid, prod, 0.0), axis=0, keepdims=True)
        return jnp.broadcast_to(mneg.astype(bf16).astype(f32), (8, TQ))

    def unit_q(pr, par, qb, mneg8):
        h = 2 * pr + par
        off = (h * DH) % 128
        t = (h * DH) // 128
        strad = off > 128 - DH
        tile = t + _sel(strad, NT5, 0)
        olp = _sel(strad, 32, _sel(t == NT5 - 1, 0, 63))
        qcols = _rows(qb, TQ)
        ra = pl.ds(_dyn(64 * t + _sel(strad, 64, 0), 32), 32)
        rb = pl.ds(_dyn(64 * t + 32, 32), 32)
        w = jnp.concatenate([qT_s[ra, qcols], qT_s[rb, qcols]], axis=0)
        r = lax.broadcasted_iota(jnp.int32, (64, TQ), 0)
        msk = ((2 * r - off + 128) & 127) < DH
        if mneg8 is None:
            other = jnp.zeros((64, TQ), u32)
        else:
            mb = pltpu.bitcast(mneg8, u32)
            other = jnp.where(r == olp, jnp.concatenate([mb] * 8, axis=0), jnp.zeros((), u32))
        qm = pltpu.bitcast(jnp.where(msk, w, other), bf16)
        return qm, tile, (par, qb, mneg8, {"rq0": 40 * pr + 16 * par, "hd": h * DH})

    def vpu_sum(info, g, j, d0, nd, init):
        par, qb, _, cache = info
        o4 = 4 * par
        if ("rq", g) not in cache:
            z8 = zbit(16 + g) * 8
            cache[("rq", g)] = pl.multiple_of(cache["rq0"] - z8 if par else cache["rq0"] + z8, 8)
        if ("ops", g, j) not in cache:
            z1 = zbit(4 * qb + j)
            gz = g + z1 if g + 1 < NGRP else g - z1
            cache[("ops", g, j)] = (
                qTf_s[pl.ds(cache[("rq", g)], VR), pl.ds(qb * TQ + 128 * j, 128)],
                kb_all[gz, pl.ds(cache["hd"], DH)].reshape(DH, 2, 8, 128))
        wf, kb = cache[("ops", g, j)]
        kb = kb[d0:d0 + nd]
        qb_ = lax.concatenate(
            [lax.broadcast_in_dim(lax.slice(wf, (o4 + d, 0), (o4 + d + 1, 128)), (1, 1, 8, 128), (2, 3))
             for d in range(d0, d0 + nd)], 0)
        prod = kb * qb_
        cuts = [(i * nd) // NCH for i in range(NCH + 1)]
        parts = [jnp.sum(prod[a:b], axis=0) for a, b in zip(cuts[:-1], cuts[1:]) if b > a]
        parts[0] = parts[0] + init
        while len(parts) > 1:
            parts = [parts[k] + parts[k + 1] if k + 1 < len(parts) else parts[k] for k in range(0, len(parts), 2)]
        return parts[0]

    def step_qk(uq, c, extra_pins):
        qm, tile, info = uq
        nm = KC - 16 if c in ASSIST else KC
        ku = k_s[tile, pl.ds(c * KC // 2, nm // 2), :]
        pins = []
        wk = WORK_AT[c]
        i = 0
        while i < len(wk):
            pos, (g, j, k) = wk[i]
            dst = (pl.ds(ASSIST[g] * KC + KC - 16, 16), slice(128 * j, 128 * (j + 1)))
            nq = 1
            i += 1
            while i < len(wk) and wk[i][0] == pos and wk[i][1][:2] == (g, j):
                nq += 1
                i += 1
            cache = info[3]
            if k == 0:
                init = info[2][None, :, 128 * j:128 * (j + 1)]
            elif ("part", g, j) in cache:
                init = cache.pop(("part", g, j))
            else:
                init = sA[dst].reshape(2, 8, 128)
            v = vpu_sum(info, g, j, 5 * k, 5 * nq, init)
            if k + nq == 4 or (c == LAG - 1 and i == len(wk)):
                sA[dst] = v.reshape(16, 128)
            if k + nq < 4:
                cache[("part", g, j)] = v
            pins.append((pos, v[0]))
            pins.append((pos, v[1]))
        pins += extra_pins
        pvpins = [v for pos, v in pins if pos == 9]
        pins = [(pos, v) for pos, v in pins if pos != 9]
        if pins:
            parts = [ku[8 * j:8 * j + 8] for j in range(nm // 16)]
            for pos, v in pins:
                parts[pos] = lax.select(tmask[0], parts[pos], pltpu.bitcast(v, u32))
            ku = jnp.concatenate(parts, axis=0)
        sA[pl.ds(c * KC, nm), :] = jnp.dot(pltpu.bitcast(ku, bf16), qm, preferred_element_type=f32)
        return pvpins

    def store_o(acc, pr, par, qb):
        orow = _dyn(pr * 40, 8)
        qcols = _rows(qb, TQ)
        if par == 0:
            l = acc[DH:DH + 1, :]
            oT_s[pl.ds(orow, VR), qcols] = acc * (1.0 / l)
        else:
            l = acc[0:1, :]
            o = acc * (1.0 / l)
            lo4 = lax.broadcasted_iota(jnp.int32, (8, TQ), 0) < 4
            mid_e = oT_s[pl.ds(orow + 16, 8), qcols]
            oT_s[pl.ds(orow + 16, 8), qcols] = jnp.where(lo4, mid_e, o[0:8])
            oT_s[pl.ds(orow + 24, 16), qcols] = o[8:24]
        return l

    new_block()
    m0 = unit_m(0, 0, 0)
    uq0 = unit_q(0, 0, 0, m0)
    for c in range(LAG):
        step_qk(uq0, c, [])

    def body(p, carry):
        ok, m_cur = carry
        new_block()
        pn = jnp.minimum(p + 1, H // 2 - 1)
        acc = None
        uq = None
        ms = {0: m_cur}
        for n in range(8 * NSTEP):
            ka, ca = divmod(n + LAG, NSTEP)
            if ca == 0 or n == 0:
                uq = unit_q(p if ka < 8 else pn, (ka % 8) // 4, ka % 4, ms[ka])
            extra = []
            if ca == MSTEP and ka < 8:
                k2 = ka + 1
                ms[k2] = unit_m(p if k2 < 8 else pn, (k2 % 8) // 4, k2 % 4)
                extra = [(9, ms[k2][:, 128 * j:128 * (j + 1)]) for j in range(TQ // 128)]
            pvpins = step_qk(uq, ca, extra)
            kb_, cb = divmod(n, NSTEP)
            par, qb = kb_ // 4, kb_ % 4
            vrow = pl.multiple_of(p * 48 + 24 * par, 8)
            pp = jnp.exp2(sA[pl.ds(cb * KC, KC), :]).astype(bf16)
            vt = vT_s[pl.ds(vrow, VR), pl.ds(cb * KC, KC)]
            if pvpins:
                v0 = vt[0:8]
                for v in pvpins:
                    v0 = lax.select(tmask[0], v0, v)
                vt = jnp.concatenate([v0, vt[8:]], axis=0)
            r = jnp.dot(vt, pp, preferred_element_type=f32)
            if cb == 0:
                acc = jnp.full((VR, TQ), zero_s[1].astype(f32), f32) + r
            else:
                acc = acc + r
            if cb == NSTEP - 1:
                l = store_o(acc, p, par, qb)
                fin = jnp.abs(acc) <= AMAX
                good = fin[0:8] & fin[8:16] & fin[16:24] & (l >= LMIN)
                ok = jnp.minimum(ok, jnp.where(good, 1.0, -1.0))
        return ok, ms[8]

    ok, _ = lax.fori_loop(0, H // 2, body, (jnp.ones((8, TQ), f32), m0))

    @pl.when(jnp.min(ok) < 0.0)
    def _fallback():
        def unit(u, c0):
            pr = u // 8
            for par in range(2):
                @pl.when((u // 4) % 2 == par)
                def _():
                    qb = u % 4
                    qm, tile, _info = unit_q(pr, par, qb, None)

                    def pass1(c, m8):
                        kk = pltpu.bitcast(k_s[tile, _rows(c, KC // 2), :], bf16)
                        s = jnp.dot(kk, qm, preferred_element_type=f32)
                        sA[_rows(c, KC), :] = s
                        return jnp.maximum(m8, jnp.max(s.reshape(KC // 8, 8, TQ), axis=0))
                    m8 = lax.fori_loop(0, NSTEP, pass1, jnp.full((8, TQ), -jnp.inf, f32))
                    m = jnp.max(m8, axis=0, keepdims=True)
                    vrow = pl.multiple_of(pr * 48 + 24 * par, 8)

                    def pass2(c, acc):
                        krows = _rows(c, KC)
                        pp = jnp.exp2(sA[krows, :] - m).astype(bf16)
                        return acc + jnp.dot(vT_s[pl.ds(vrow, VR), krows], pp, preferred_element_type=f32)
                    acc = lax.fori_loop(0, NSTEP, pass2, jnp.zeros((VR, TQ), f32))
                    store_o(acc, pr, par, qb)
            return c0
        lax.fori_loop(0, H * NQ, unit, 0)

    wo_copy.wait()
    w1_copy.wait()
    w2_copy.wait()
    b1_copy.wait()
    b2_copy.wait()

    def out_copy(g):
        slot = g % (2 * NH3)
        return pltpu.make_async_copy(out_s.at[slot], o_hbm.at[_rows(g, T3), :], sem_o.at[slot])

    def p3(trip, c):
        @pl.when(trip >= 2)
        def _():
            for k in range(NH3):
                out_copy((trip - 2) * NH3 + k).wait()

        b1 = b1_ref[...].reshape(1, F).astype(f32)
        b2 = b2_ref[...].reshape(1, D).astype(f32)
        hres = []
        for k in range(NH3):
            rows = _rows(trip * NH3 + k, T3)
            oT = oT_s[:, rows].astype(bf16)
            attn = lax.dot_general(oT, wo_s[...], TN, preferred_element_type=f32)
            hres.append(x_s[rows, :].astype(f32) + attn)
        act = []
        for k in range(NH3):
            hn = _ln(hres[k]).astype(bf16)
            a = jnp.dot(hn, w1_s[...], preferred_element_type=f32) + b1
            act.append(_gelu(a).astype(bf16))
        for k in range(NH3):
            g = trip * NH3 + k
            y = jnp.dot(act[k], w2_s[...], preferred_element_type=f32) + b2
            out_s[g % (2 * NH3)] = (hres[k] + y).astype(bf16)
            out_copy(g).start()
        return c

    lax.fori_loop(0, S // (T3 * NH3), p3, 0)
    for g in range(S // T3 - 2 * NH3, S // T3):
        out_copy(g).wait()


@jax.jit
def pallas_sequential_preLN__softmax_full_mha__dense_activation_gelu__prompt_kernel(
    A_x: jax.Array,
    A_wqkv: jax.Array,
    A_wo: jax.Array,
    B_x: jax.Array,
    B_w1: jax.Array,
    B_b1: jax.Array,
    B_w2: jax.Array,
    B_b2: jax.Array,
):
    anyspec = pl.BlockSpec(memory_space=pl.ANY)
    out = pl.pallas_call(
        _kernel,
        in_specs=[anyspec] * 7,
        out_specs=anyspec,
        out_shape=jax.ShapeDtypeStruct((S, D), bf16),
        scratch_shapes=[
            pltpu.VMEM((S, D), bf16),
            pltpu.VMEM((D, 3 * D), bf16),
            pltpu.VMEM((D, D), bf16),
            pltpu.VMEM((D, F), bf16),
            pltpu.VMEM((F, D), bf16),
            pltpu.VMEM((NTILE, S // 2, 128), u32),
            pltpu.VMEM((D // 2, S), u32),
            pltpu.VMEM((D, S), f32),
            pltpu.VMEM((DV, S), f32),
            pltpu.VMEM((S, TQ), f32),
            pltpu.VMEM((D, S), f32),
            pltpu.VMEM((2 * NH3, T3, D), bf16),
            pltpu.VMEM((F,), bf16),
            pltpu.VMEM((D,), bf16),
            pltpu.VMEM((1, 2944), f32),
            pltpu.VMEM((NGRP, D, 16, 128), f32),
            pltpu.VMEM((D, 128), f32),
            pltpu.SMEM((64,), jnp.int32),
            pltpu.SemaphoreType.DMA((N1,)),
            pltpu.SemaphoreType.DMA((9,)),
            pltpu.SemaphoreType.DMA((2 * NH3,)),
        ],
        compiler_params=pltpu.CompilerParams(vmem_limit_bytes=116 * 1024 * 1024),
    )(A_x.reshape(S, D), A_wqkv, A_wo, B_w1, B_w2, B_b1, B_b2)
    return out.reshape(1, S, D)
```
